```python
import os as _os
_os.environ.setdefault("JAX_PLATFORMS", "cpu")
import jax
import jax.numpy as jnp

def _softmax(x, axis=-1):
    return jax.nn.softmax(x, axis=axis)
def _gelu(x):
    return jax.nn.gelu(x, approximate=True)
def _silu(x):
    return jax.nn.silu(x)
def _sigmoid(x):
    return jax.nn.sigmoid(x)
def _layernorm(x, axis=-1, eps=1e-5):
    m = jnp.mean(x, axis=axis, keepdims=True)
    v = jnp.var(x, axis=axis, keepdims=True)
    return (x - m) / jnp.sqrt(v + eps)
def _scatter_add(tgt, idx, src, axis=0):
    return tgt.at[idx].add(src)
def _segment_sum(src, seg, n):
    return jax.ops.segment_sum(src, seg, n)
class _Rng:
    def __init__(self, key):
        self._k = key
    def _next(self):
        self._k, sub = jax.random.split(self._k)
        return sub
    def normal(self, shape):
        return jax.random.normal(self._next(), shape, dtype=jnp.bfloat16)
    def randint(self, lo, hi, shape):
        return jax.random.randint(self._next(), shape, lo, hi, dtype=jnp.int32)
    def uniform(self, shape, lo=0.0, hi=1.0):
        return jax.random.uniform(self._next(), shape, jnp.bfloat16, lo, hi)
    def permutation(self, n):
        return jax.random.permutation(self._next(), n)


kernel_name = 'sequential_preLN__softmax_full_mha__dense_activation_squared_relu__prompt'

def setup_inputs():
    _rng = _Rng(jax.random.key(int.from_bytes(__import__("os").urandom(4), "little")))
    _w = (lambda a: (lambda t: t.astype(jnp.bfloat16) if jnp.issubdtype(t.dtype, jnp.floating) else t)(jnp.asarray(a)))
    def _A_setup():
        B, S, D = 1, 2048, 640
        return {
            "x": _w((lambda *s: _rng.normal(s) * 0.05)(B, S, D)),
            "wqkv": _w((lambda *s: _rng.normal(s) * 0.05)(D, 3 * D)),
            "wo": _w((lambda *s: _rng.normal(s) * 0.05)(D, D)),
        }
    _A_in = _A_setup()

    def _B_setup():
        B, S, D, F = 1, 2048, 640, 1536
        return {
            "x": _w((lambda *s: _rng.normal(s) * 0.05)(B, S, D)),
            "w1": _w((lambda *s: _rng.normal(s) * 0.05)(D, F)),
            "b1": _w((lambda *s: _rng.normal(s) * 0.05)(F)),
            "w2": _w((lambda *s: _rng.normal(s) * 0.05)(F, D)),
            "b2": _w((lambda *s: _rng.normal(s) * 0.05)(D)),
        }
    _B_in = _B_setup()

    return {
        "A_x": _A_in["x"],
        "A_wqkv": _A_in["wqkv"],
        "A_wo": _A_in["wo"],
        "B_x": _B_in["x"],
        "B_w1": _B_in["w1"],
        "B_b1": _B_in["b1"],
        "B_w2": _B_in["w2"],
        "B_b2": _B_in["b2"],
    }

def reference(A_x, A_wqkv, A_wo, B_x, B_w1, B_b1, B_w2, B_b2):
    def _A_ref(x, wqkv, wo):
        B, S, D = x.shape
        H = 32; Dh = D // H
        qkv = (lambda x, *d: x.transpose(*d))((x @ wqkv).reshape(B, S, 3, H, Dh), 2, 0, 3, 1, 4)
        q, k, v = qkv[0], qkv[1], qkv[2]
        scale = Dh ** -0.5
        scores = jnp.einsum("bhqd,bhkd->bhqk", q, k) * scale
        p = _softmax(scores, axis=-1)
        o = jnp.einsum("bhqk,bhkd->bhqd", p, v)
        return (lambda x, *d: x.transpose(*d))(o, 0, 2, 1, 3).reshape(B, S, D) @ wo

    def _B_ref(x, w1, b1, w2, b2):
        h = jnp.einsum("bsd,df->bsf", x, w1) + b1
        zero = jnp.zeros_like(h)
        r = jnp.where(h > zero, h, zero)
        h = r * r
        out = jnp.einsum("bsf,fd->bsd", h, w2) + b2
        return out

    x = A_x
    h = x + _A_ref(_layernorm(x, axis=-1), A_wqkv, A_wo)
    h2 = h + _B_ref(_layernorm(h, axis=-1), B_w1, B_b1, B_w2, B_b2)
    return h2
```

```python
import contextlib
import jax
import jax.numpy as jnp
from jax import lax
import jax.experimental.pallas as pl
import jax.experimental.pallas.tpu as pltpu

F32, BF16, I32 = jnp.float32, jnp.bfloat16, jnp.int32

S, D, F, H = 2048, 640, 1536, 32
DH = D // H
LANE = 128
NT = S // LANE
RB = 512
NB = S // RB
TPB = RB // LANE
KD = 32
VR = 24
CK = 128
NCK = S // CK
EPS = 1e-5
QSCALE = float(DH ** -0.5 * 1.4426950408889634)

CFG = dict(
    noff=24,
    gb=4, pa=1, pb=1, dsplit=1, order="epvq", exlead=1, qlead=0, flags="D",
    mode="T",
    hpb=1,
    skip=0, bspan=90, vspan=100, vstart=0, pack=0,
)


def _ln(x):
    mean = jnp.mean(x, axis=-1, keepdims=True)
    xc = x - mean
    var = jnp.mean(xc * xc, axis=-1, keepdims=True)
    return xc * lax.rsqrt(var + EPS)


def _dot(a, b):
    return jnp.dot(a, b, preferred_element_type=F32)


def _lanes(u, n=1):
    return slice(u * LANE, (u + n) * LANE)


def _make_kernel(cfg):
    noff, gb, pa, pb = cfg["noff"], cfg["gb"], cfg["pa"], cfg["pb"]
    hpb = cfg["hpb"]
    true_max = cfg["mode"] == "T"
    pack = bool(cfg["pack"]) and not true_max
    koff = 8 * noff
    kmx = S - koff
    bounds = [16 * ((kmx // 16) * t // NCK) for t in range(NCK + 1)]

    scope = jax.named_scope if cfg.get('scopes') else (lambda name: contextlib.nullcontext())

    def kernel(x_hbm, wqkv_hbm, wo_hbm, w1_hbm, b1_hbm, w2_hbm, b2_hbm, o_hbm,
               xv, wqkv, wo, w1, w2, xn, kw, ko, qw, qh, vw, oraw, hres, hn, ostage,
               sem_x, sem_w, sem_o, *bufs):
        nh = 2 * hpb
        b1, b2 = bufs[-2:]
        sbuf = [bufs[p * hpb:(p + 1) * hpb] for p in range(2)]
        mbuf = [bufs[nh + p * hpb:nh + (p + 1) * hpb] for p in range(2)]
        kb = [bufs[2 * nh + p * hpb:2 * nh + (p + 1) * hpb] for p in range(2)]
        qb = [bufs[3 * nh + p * hpb:3 * nh + (p + 1) * hpb] for p in range(2)]

        def x_copy(i):
            return pltpu.make_async_copy(x_hbm.at[pl.ds(i * RB, RB)], xv.at[i], sem_x.at[i])

        def o_copy(i):
            return pltpu.make_async_copy(ostage.at[i], o_hbm.at[pl.ds(i * RB, RB)], sem_o.at[i])

        w_copies = [pltpu.make_async_copy(src, dst, sem_w.at[n]) for n, (src, dst) in enumerate(
            [(wqkv_hbm, wqkv), (wo_hbm, wo), (w1_hbm, w1), (b1_hbm, b1), (w2_hbm, w2), (b2_hbm, b2)])]

        x_copy(0).start()
        w_copies[0].start()
        for i in range(1, NB):
            x_copy(i).start()
        for c in w_copies[1:]:
            c.start()

        x_copy(0).wait()
        xn[0] = _ln(xv[0].astype(F32)).astype(BF16)
        w_copies[0].wait()

        def project(i, last):
            a = xn[i]
            row = lax.broadcasted_iota(I32, (KD, RB), 0)
            row8 = lax.broadcasted_iota(I32, (8, RB), 0)
            qt = (_dot(a, wqkv[:, 0:D]) * QSCALE).T
            for h in range(H):
                w0 = 16 * (DH * h // 16)
                lo = DH * h - w0
                win = jnp.where((row >= lo) & (row < lo + DH), qt[w0:w0 + KD], 0.0)
                qw[h, i] = pltpu.bitcast(win.astype(BF16), I32)
                if noff:
                    b0 = 8 * (DH * h // 8)
                    qh[h, i] = qt[b0:b0 + VR]
            k = _dot(a, wqkv[:, D:2 * D])
            rows = RB - koff if last else RB
            kp = pltpu.bitcast(k[:rows].astype(BF16), I32)
            for h in range(H):
                w0 = 16 * (DH * h // 16)
                if last:
                    kw[h, (NB - 1) * RB // 2:kmx // 2, :] = kp[:, w0:w0 + KD]
                    if noff:
                        ko[h] = k[rows:, DH * h:DH * (h + 1)]
                else:
                    kw[h, pl.ds(pl.multiple_of(i * (RB // 2), RB // 2), RB // 2), :] = kp[:, w0:w0 + KD]
            vt = _dot(a, wqkv[:, 2 * D:3 * D]).T
            for h in range(H):
                b0 = 8 * (DH * h // 8)
                if h % 2 == 0:
                    vw[h, i, 0:16] = vt[b0:b0 + 16]
                    vw[h, i, 16:24] = jnp.where(row8 < 4, vt[b0 + 16:b0 + 24], 1.0)
                else:
                    vw[h, i, 0:8] = jnp.where(row8 < 4, 1.0, vt[b0:b0 + 8])
                    vw[h, i, 8:24] = vt[b0 + 8:b0 + 24]

        def phase1(i, carry):
            x_copy(i + 1).wait()
            xn[i + 1] = _ln(xv[i + 1].astype(F32)).astype(BF16)
            project(i, False)
            return carry

        with scope('p1loop'):
            lax.fori_loop(0, NB - 1, phase1, 0)
        with scope('p1last'):
            project(NB - 1, True)

        def attention(hq, hv, hb, par):
            nxt, cur = par, 1 - par
            mx, acc, pend, vacc = {}, {}, {}, {}

            def upd(g, u, s):
                if true_max:
                    t = jnp.max(s.reshape(-1, 8, LANE), axis=0)
                    mx[g, u] = t if (g, u) not in mx else jnp.maximum(mx[g, u], t)

            def put(g, a, b, u, s):
                n = s.shape[1] // LANE
                for w in range(n):
                    upd(g, u + w, s[:, _lanes(w)])
                if pack:
                    sbuf[nxt][g][a // 2:b // 2, _lanes(u, n)] = pltpu.bitcast(jnp.exp2(s).astype(BF16), I32)
                else:
                    sbuf[nxt][g][a:b, _lanes(u, n)] = s

            def qk(g, c, u):
                a, b = bounds[c], bounds[c + 1]
                kk = pltpu.bitcast(kw[hq + g, a // 2:b // 2, :], BF16)
                qq = pltpu.bitcast(qw[hq + g, u // TPB, :, _lanes(u % TPB)], BF16)
                put(g, a, b, u, _dot(kk, qq))

            def vp(g, a0, u, d0, d1):
                ac = vacc.get((g, a0, u), [None] * pa)
                for d in range(d0, d1):
                    qd = qb[nxt][g][d, :, _lanes(u, pb)]
                    for a in range(pa):
                        kv = kb[nxt][g][d, (a0 + a) * 8:(a0 + a + 1) * 8, :]
                        t = (jnp.concatenate([kv] * pb, axis=1) if pb > 1 else kv) * qd
                        ac[a] = t if ac[a] is None else ac[a] + t
                vacc[g, a0, u] = ac
                if d1 == DH:
                    s = ac[0] if pa == 1 else jnp.concatenate(ac, axis=0)
                    put(g, kmx + a0 * 8, kmx + (a0 + pa) * 8, u, s)

            def ex(g, c, u):
                if pack:
                    pend[g, c, u] = pltpu.bitcast(sbuf[cur][g][c * CK // 2:(c + 1) * CK // 2, _lanes(u)], BF16)
                    return
                s = sbuf[cur][g][c * CK:(c + 1) * CK, _lanes(u)]
                if true_max:
                    s = (s.reshape(CK // 8, 8, LANE) - mbuf[cur][g][:, _lanes(u)][None]).reshape(CK, LANE)
                pend[g, c, u] = jnp.exp2(s)

            def pv(g, c, u):
                v = vw[hv + g, c // TPB, :, _lanes(c % TPB)]
                o = _dot(v, pend.pop((g, c, u)))
                acc[g, u] = o if c == 0 else acc[g, u] + o
                if c == NCK - 1:
                    oraw[hv + g, u // TPB, :, _lanes(u % TPB)] = acc[g, u]

            def fin(g, u):
                m = jnp.max(mx[g, u], axis=0, keepdims=True)
                mbuf[nxt][g][:, _lanes(u)] = jnp.broadcast_to(m, (8, LANE))

            def bk(g, a):
                kk = ko[hb + g, a * 8:(a + 1) * 8, :]
                for d in range(DH):
                    kb[cur][g][d, a * 8:(a + 1) * 8, :] = jnp.broadcast_to(kk[:, d:d + 1], (8, LANE))

            def bq(g, u):
                odd = (g if hpb == 2 else cur) % 2
                q = qh[hb + g, u // TPB, :, _lanes(u % TPB)]
                for d in range(DH):
                    r = d + 4 * odd
                    qb[cur][g][d, :, _lanes(u)] = jnp.broadcast_to(q[r:r + 1, :], (8, LANE))

            order, ev = cfg["order"], []
            total = hpb * NT * NCK
            for g in range(hpb):
                for j in range(NT // gb):
                    t0 = (g * (NT // gb) + j) * NCK * gb
                    for c in range(NCK):
                        for w in range(gb):
                            t, u = t0 + c * gb + w, j * gb + w
                            if hv is not None:
                                ev.append((t - cfg["exlead"], order.index("e"), ex, (g, c, u)))
                                ev.append((t, order.index("p"), pv, (g, c, u)))
                            if hq is not None:
                                ev.append((t - cfg["qlead"], order.index("q"), qk, (g, c, u)))
                    if hq is None:
                        continue
                    ds = cfg["dsplit"]
                    ps = [(g, a0, j * gb + w, DH * s // ds, DH * (s + 1) // ds)
                          for a0 in range(0, noff, pa) for w in range(0, gb, pb) for s in range(ds)]
                    for n, p in enumerate(ps):
                        t = (t0 + NCK * gb * (n + 0.5) / len(ps)) * cfg["vspan"] / 100 + cfg["vstart"]
                        ev.append((t, order.index("v"), vp, p))
                    if true_max:
                        for w in range(gb):
                            ev.append((t0 + NCK * gb + max(cfg["vstart"], 0) + w, 9, fin, (g, j * gb + w)))
            if hb is not None and noff:
                for fn, cnt in [((bk, noff), (bq, NT)), ((bk, noff),), ((bq, NT),), ()][cfg['skip']]:
                    for n in range(hpb * cnt):
                        ev.append((total * cfg["bspan"] / 100 * (n + 0.5) / (hpb * cnt), 8, fn, divmod(n, cnt)))
            ev.sort(key=lambda e: (e[0], e[1]))
            for e in ev:
                e[2](*e[3])

        steps = H // hpb
        with scope('att0'):
            attention(None, None, 0, 1)
            attention(0, None, hpb, 0)

        def phase2(i, carry):
            for par in range(2):
                @pl.when(i % 2 == par)
                def _():
                    attention(i * hpb, (i - 1) * hpb, jnp.minimum(i + 1, steps - 1) * hpb, par)
            return carry

        with scope('attloop'):
            lax.fori_loop(1, steps, phase2, 0)
        with scope('attlast'):
            attention(None, (steps - 1) * hpb, None, steps % 2)

        for c in w_copies[1:]:
            c.wait()

        def mix(i):
            row8 = lax.broadcasted_iota(I32, (8, RB), 0)
            parts = []
            for h in range(0, H, 2):
                e, o = oraw[h, i], oraw[h + 1, i]
                e = e * (1.0 / e[20:21])
                o = o * (1.0 / o[0:1])
                parts += [e[0:16], jnp.where(row8 < 4, e[16:24], o[0:8]), o[8:24]]
            att = jnp.concatenate(parts, axis=0).T.astype(BF16)
            hh = xv[i].astype(F32) + _dot(att, wo[...])
            hres[i] = hh
            hn[i] = _ln(hh).astype(BF16)

        def ffn(i):
            g = _dot(hn[i], w1[...]) + b1[...].astype(F32).reshape(1, F)
            r = jnp.maximum(g, 0.0)
            out = hres[i] + (_dot((r * r).astype(BF16), w2[...]) + b2[...].astype(F32).reshape(1, D))
            ostage[i] = out.astype(BF16)
            o_copy(i).start()

        with scope('mix0'):
            mix(0)

        def phase3(i, carry):
            mix(i + 1)
            ffn(i)
            return carry

        with scope('p3loop'):
            lax.fori_loop(0, NB - 1, phase3, 0)
        with scope('p3last'):
            ffn(NB - 1)
        for i in range(NB):
            o_copy(i).wait()

    nh = 2 * hpb
    scratch = [
        pltpu.VMEM((NB, RB, D), BF16),
        pltpu.VMEM((D, 3 * D), BF16),
        pltpu.VMEM((D, D), BF16),
        pltpu.VMEM((D, F), BF16),
        pltpu.VMEM((F, D), BF16),
        pltpu.VMEM((NB, RB, D), BF16),
        pltpu.VMEM((H, kmx // 2, KD), I32),
        pltpu.VMEM((H, max(koff, 8), DH), F32),
        pltpu.VMEM((H, NB, KD // 2, RB), I32),
        pltpu.VMEM((H, NB, VR, RB), F32),
        pltpu.VMEM((H, NB, VR, RB), F32),
        pltpu.VMEM((H, NB, VR, RB), F32),
        pltpu.VMEM((NB, RB, D), F32),
        pltpu.VMEM((NB, RB, D), BF16),
        pltpu.VMEM((NB, RB, D), BF16),
        pltpu.SemaphoreType.DMA((NB,)),
        pltpu.SemaphoreType.DMA((6,)),
        pltpu.SemaphoreType.DMA((NB,)),
    ]
    scratch += [pltpu.VMEM((S // 2, S), I32) if pack else pltpu.VMEM((S, S), F32)] * nh
    scratch += [pltpu.VMEM((8, S), F32)] * nh
    scratch += [pltpu.VMEM((DH, max(koff, 8), LANE), F32)] * nh
    scratch += [pltpu.VMEM((DH, 8, S), F32)] * nh
    scratch += [pltpu.VMEM((F,), BF16), pltpu.VMEM((D,), BF16)]
    return kernel, scratch


def _run(cfg, A_x, A_wqkv, A_wo, B_w1, B_b1, B_w2, B_b2):
    kernel, scratch = _make_kernel(cfg)
    flags = {}
    if "D" in cfg["flags"]:
        flags["XLA_TPU_EVENLY_DISTRIBUTE_CRITICAL_NODES"] = True
    if "L" in cfg["flags"]:
        flags["XLA_TPU_FORCE_LP_LLO_SCHEDULER"] = True
    out = pl.pallas_call(
        kernel,
        out_shape=jax.ShapeDtypeStruct((S, D), BF16),
        in_specs=[pl.BlockSpec(memory_space=pl.ANY)] * 7,
        out_specs=pl.BlockSpec(memory_space=pl.ANY),
        scratch_shapes=scratch,
        compiler_params=pltpu.CompilerParams(vmem_limit_bytes=126 * 2**20, flags=flags or None),
    )(A_x.reshape(S, D), A_wqkv, A_wo, B_w1, B_b1, B_w2, B_b2)
    return out.reshape(1, S, D)


@jax.jit
def pallas_sequential_preLN__softmax_full_mha__dense_activation_squared_relu__prompt_kernel(
    A_x, A_wqkv, A_wo, B_x, B_w1, B_b1, B_w2, B_b2,
):
    del B_x
    return _run(CFG, A_x, A_wqkv, A_wo, B_w1, B_b1, B_w2, B_b2)
```

```python
import functools

import jax
import jax.numpy as jnp
from jax import lax
import jax.experimental.pallas as pl
import jax.experimental.pallas.tpu as pltpu

F32, BF16, I32 = jnp.float32, jnp.bfloat16, jnp.int32

S, D, F, H = 2048, 640, 1536, 32
DH = D // H
LANE = 128
NT = S // LANE
RB = 512
NB = S // RB
TPB = RB // LANE
KD = 32
VR = 24
EPS = 1e-5
QSCALE = float(DH ** -0.5 * 1.4426950408889634)
SUM_MIN, SUM_MAX = 2.0 ** -40, 2.0 ** 60

CFG = dict(noff=34, gb=16, dsplit=10, exlead=4.0, qlead=3.5, bstart=20, bspan=80, qstart=30, qspan=60,
           vspan=99.0, vstart=3.0, vrot=3, lh=8, g1=85, g2=95, c2=100, force=0, only=0, first=0)

_A_TERMS = (((1, 0), (1, 3)), ((1, 3),), ((1, 0), (1, 1)), ((1, 1), (-1, 3)), ((1, 2), (1, 3)), ((1, 0),), ((1, 2), (-1, 0)))
_B_TERMS = (((1, 0), (1, 3)), ((1, 2), (-1, 0)), ((1, 3),), ((1, 2), (1, 3)), ((1, 0),), ((1, 1), (-1, 3)), ((1, 0), (1, 1)))
_C_TERMS = (((1, 0), (1, 3)), ((1, 0), (1, 2)), ((-1, 0), (1, 1)), ((1, 0),), ((1, 2), (-1, 3)), ((1, 1), (1, 3)), ((1, 3),))


def _ln(x):
    mean = jnp.mean(x, axis=-1, keepdims=True)
    xc = x - mean
    var = jnp.mean(xc * xc, axis=-1, keepdims=True)
    return xc * lax.rsqrt(var + EPS)


def _dot(a, b):
    return jnp.dot(a, b, preferred_element_type=F32)


def _lanes(u):
    return slice(u * LANE, (u + 1) * LANE)


def _pack(v):
    return pltpu.bitcast(v.astype(BF16), I32)


def _unpack(v):
    return pltpu.bitcast(v, BF16)


def _half(a, b):
    return slice(a // 2, b // 2)


def _operands(blocks, terms, level):
    if level == 0:
        return [blocks[0][0]]
    n = len(blocks) // 2
    out = []
    for (_, first), *rest in terms:
        def combine(i, j):
            val = blocks[first // 2 * n + i][first % 2 * n + j]
            for sign, q in rest:
                other = blocks[q // 2 * n + i][q % 2 * n + j]
                val = val + other if sign > 0 else val - other
            return val
        out += _operands([[combine(i, j) for j in range(n)] for i in range(n)], terms, level - 1)
    return out


def _combine(product):
    out = {}
    for r, term in enumerate(_C_TERMS):
        grid = product(r)
        n = len(grid)
        for sign, q in term:
            for i in range(n):
                for j in range(n):
                    key = (q // 2 * n + i, q % 2 * n + j)
                    if key not in out:
                        out[key] = grid[i][j]
                    else:
                        out[key] = out[key] + grid[i][j] if sign > 0 else out[key] - grid[i][j]
    return [[out[i, j] for j in range(2 * n)] for i in range(2 * n)]


class _Filler:
    def __init__(self, parent=None):
        self.jobs, self.now, self.parent = [], 0, parent

    def add(self, jobs, start, stop):
        self.jobs += [(start + (stop - start) * (n + 0.5) / len(jobs), job) for n, job in enumerate(jobs)]
        self.jobs.sort(key=lambda e: e[0])

    def tick(self, work):
        self.now += work
        if self.parent is not None:
            self.parent.tick(work)
        while self.jobs and self.jobs[0][0] <= self.now:
            self.jobs.pop(0)[1]()

    def flush(self):
        while self.jobs:
            self.jobs.pop(0)[1]()


class _Linear:
    def __init__(self, k, n, level):
        self.k, self.n, self.level, self.q = k, n, level, 2 ** level
        self.kq = k // (LANE * self.q)
        self.nq = n // (LANE * self.q)
        self.rows = RB // self.q
        self.work = (7 ** level * self.rows * self.kq * self.nq
                     + RB * ((k // LANE) * (n // LANE) - self.kq * self.nq * self.q ** 2))

    def weight_scratch(self):
        return pltpu.VMEM((7 ** self.level, self.kq * LANE // 2, self.nq * LANE), I32)

    def input_scratch(self, slots):
        return pltpu.VMEM((slots, 7 ** self.level, self.rows // 2, self.kq * LANE), I32)

    def weight_jobs(self, w_ref, op_ref, groups=None):
        part = self.kq * LANE

        def job(r0, j):
            blocks = [[w_ref[a * part + r0:a * part + r0 + 16, _lanes(b * self.nq + j)].astype(F32)
                       for b in range(self.q)] for a in range(self.q)]
            for r, op in enumerate(_operands(blocks, _B_TERMS, self.level)):
                op_ref.at[r][_half(r0, r0 + 16), _lanes(j)] = _pack(op)
        return [functools.partial(job, r0, j) for j in (range(self.nq) if groups is None else groups)
                for r0 in range(0, part, 16)]

    def put_input(self, block, op_ref, r0, r1, tiles=None):
        for kt in range(self.kq) if tiles is None else tiles:
            blocks = [[block(i, b * self.kq + kt) for b in range(self.q)] for i in range(self.q)]
            for r, op in enumerate(_operands(blocks, _A_TERMS, self.level)):
                op_ref.at[r][_half(r0, r1), _lanes(kt)] = _pack(op)

    def columns(self, a_ref, aop_ref, w_ref, wop_ref, filler, step):
        def dot(a, b):
            out = _dot(a, b)
            filler.tick(a.shape[0] * a.shape[1] // LANE)
            return out

        def direct(t, k0):
            return jnp.concatenate([dot(_unpack(a_ref[_half(m, m + step), k0:self.k]), w_ref[k0:self.k, _lanes(t)])
                                    for m in range(0, RB, step)], axis=0)

        k0 = self.kq * self.q * LANE
        for j in range(self.nq):
            def product(r):
                return [[dot(_unpack(aop_ref[r]), _unpack(wop_ref[r, :, _lanes(j)]))]]
            if self.level == 1:
                grid = _combine(product)
            else:
                grid = _combine(lambda r: _combine(lambda s: product(7 * r + s)))
            out = {}
            for b in range(self.q):
                t = b * self.nq + j
                out[t] = jnp.concatenate([row[b] for row in grid], axis=0)
                if k0 < self.k:
                    out[t] = out[t] + direct(t, k0)
            yield out
        for t in range(self.nq * self.q, self.n // LANE):
            yield {t: direct(t, 0)}


def _run(cfg, A_x, A_wqkv, A_wo, B_w1, B_b1, B_w2, B_b2):
    vpu_keys = 8 * cfg["noff"]
    mxu_keys = S - vpu_keys
    kpad = -(-vpu_keys // LANE) * LANE
    early = 4
    qkv_mm, out_mm = _Linear(D, 3 * D, 1), _Linear(D, D, 1)
    up_mm, down_mm = _Linear(D, F, 2), _Linear(F, D, 1)

    def kernel(x_hbm, wqkv_hbm, wo_hbm, w1_hbm, b1_hbm, w2_hbm, b2_hbm, o_hbm,
               xv, wqkv, wo, w1, w2, wqkv_op, wo_op, w1_op, w2_op, xn, xn_op, hn_op, att, att_op, act, act_op,
               hres, kw, kt, qw, vw, oraw, seen, p0, p1, kb0, kb1, qb0, qb1, b1, b2, sem_x, sem_w, sem_o):
        probs, kb, qb = (p0, p1), (kb0, kb1), (qb0, qb1)

        def x_copy(i):
            return pltpu.make_async_copy(x_hbm.at[pl.ds(i * RB, RB)], xv.at[i], sem_x.at[i])

        def o_copy(i, t):
            return pltpu.make_async_copy(xv.at[i, :, _lanes(t)], o_hbm.at[pl.ds(i * RB, RB), _lanes(t)],
                                         sem_o.at[i * (D // LANE) + t])

        half = qkv_mm.nq * LANE
        spans = ((0, early * LANE), (half, half + early * LANE), (early * LANE, half), (half + early * LANE, 3 * D))
        pairs = [(wqkv_hbm.at[:, a:b], wqkv.at[:, a:b]) for a, b in spans]
        pairs += [(wo_hbm, wo), (w1_hbm, w1), (w2_hbm, w2), (b1_hbm, b1), (b2_hbm, b2)]
        w_copies = [pltpu.make_async_copy(src, dst, sem_w.at[n]) for n, (src, dst) in enumerate(pairs)]

        def norm_jobs(src_ref, slot, mm, op_ref, step):
            def job(r):
                ys = []
                for i in range(mm.q):
                    a = i * mm.rows + r
                    ys.append(_ln(src_ref[a:a + step, :].astype(F32)))
                    xn.at[slot][_half(a, a + step), :] = _pack(ys[i])
                mm.put_input(lambda i, t: ys[i][:, _lanes(t)], op_ref.at[slot], r, r + step)
            return [functools.partial(job, r) for r in range(0, mm.rows, step)]

        def project(i, jobs, step, hook=None):
            filler = _Filler()
            for part in jobs:
                if hook is None:
                    filler.add(part, 0, qkv_mm.work * 0.98)
                else:
                    filler.add(part, qkv_mm.work * (early + 0.1) / qkv_mm.nq, qkv_mm.work * 0.94)
            row = lax.broadcasted_iota(I32, (KD, RB), 0)
            row8 = lax.broadcasted_iota(I32, (8, RB), 0)
            nd = D // LANE
            tiles, todo = {}, [(part, h) for part in range(3) for h in range(H)]

            def window(part, start, size, axis):
                pieces = []
                for t in range(start // LANE, (min(start + size, D) - 1) // LANE + 1):
                    a, b = max(start - t * LANE, 0), min(start + size - t * LANE, LANE)
                    pieces.append(lax.slice_in_dim(tiles[part, t], a, b, axis=axis))
                if start + size > D:
                    pieces.append(jnp.zeros_like(lax.slice_in_dim(pieces[0], 0, start + size - D, axis=axis)))
                return pieces[0] if len(pieces) == 1 else jnp.concatenate(pieces, axis=axis)

            for n, res in enumerate(qkv_mm.columns(xn.at[i % 2], xn_op.at[i % 2], wqkv, wqkv_op, filler, step)):
                if hook is not None and n == early - 1:
                    hook()
                for t, val in res.items():
                    if t // nd == 0:
                        tiles[0, t % nd] = (val * QSCALE).T
                    elif t // nd == 1:
                        tiles[1, t % nd] = _pack(val)
                        if i == NB - 1:
                            tiles[3, t % nd] = val[RB - kpad:].T
                    else:
                        tiles[2, t % nd] = val.T
                for part, h in list(todo):
                    b0 = 8 * (DH * h // 8)
                    if (part, b0 // LANE) not in tiles or (part, (min(b0 + KD, D) - 1) // LANE) not in tiles:
                        continue
                    todo.remove((part, h))
                    if part == 0:
                        lo = DH * h - b0
                        qw.at[h, i][...] = _pack(jnp.where((row >= lo) & (row < lo + DH), window(0, b0, KD, 0), 0.0))
                    elif part == 1:
                        kw[h, _half(i * RB, (i + 1) * RB), :] = window(1, b0, KD, 1)
                        if i == NB - 1:
                            kt[h] = window(3, b0, VR, 0)
                    elif h % 2 == 0:
                        vw[h, i, 0:16] = window(2, b0, 16, 0)
                        vw[h, i, 16:24] = jnp.where(row8 < 4, window(2, b0 + 16, 8, 0), 1.0)
                    else:
                        vw[h, i, 0:8] = jnp.where(row8 < 4, 1.0, window(2, b0, 8, 0))
                        vw[h, i, 8:24] = window(2, b0 + 8, 16, 0)
            assert not todo
            filler.flush()

        def late_weights():
            w_copies[2].wait()
            w_copies[3].wait()
            x_copy(1).wait()
            for i in range(2, NB):
                x_copy(i).start()
            for job in qkv_mm.weight_jobs(wqkv, wqkv_op, range(early, qkv_mm.nq)):
                job()

        def first_blocks(n, carry):
            @pl.when(n == 0)
            def _():
                project(0, [norm_jobs(xv.at[1], 1, qkv_mm, xn_op, 32)], 256, late_weights)

            @pl.when(n < 1)
            def _():
                for i in range(2, NB):
                    x_copy(i).wait()
                for c in w_copies[4:]:
                    c.start()

            @pl.when(n != 1)
            def _():
                for i in range(1, NB - 1):
                    project(i, [norm_jobs(xv.at[i + 1], (i + 1) % 2, qkv_mm, xn_op, 16)], 128)

            @pl.when(n + 1 == 1)
            def _():
                for c in w_copies[4:]:
                    c.wait()
            return carry

        up_jobs = up_mm.weight_jobs(w1, w1_op)
        cut = len(up_jobs) * cfg["c2"] // 100
        if cfg["only"] == 0:
            x_copy(0).start()
            w_copies[0].start()
            w_copies[1].start()
            x_copy(0).wait()
            w_copies[2].start()
            w_copies[3].start()
            x_copy(1).start()
            for job in norm_jobs(xv.at[0], 0, qkv_mm, xn_op, 64):
                job()
            w_copies[0].wait()
            w_copies[1].wait()
            for job in qkv_mm.weight_jobs(wqkv, wqkv_op, range(early)):
                job()
            lax.fori_loop(0, 2, first_blocks, 0)
            project(NB - 1, [out_mm.weight_jobs(wo, wo_op), down_mm.weight_jobs(w2, w2_op), up_jobs[:cut]], 128)

        def attention(new, old, nxt, par, group):
            acc, pend, vacc = {}, {}, {}
            shared = old is not None
            bounds = [16 * ((mxu_keys if shared else S) // 16 * c // NT) for c in range(NT + 1)]

            def put(a, b, u, s):
                probs[par][_half(a, b), _lanes(u)] = _pack(jnp.exp2(s))

            def mxu_scores(c, u):
                k_ref, q_ref = new
                a, b = bounds[c], bounds[c + 1]
                put(a, b, u, _dot(_unpack(k_ref[_half(a, b), :]), _unpack(q_ref[u // TPB, :, _lanes(u % TPB)])))

            def vpu_scores(a0, u, d0, d1):
                sums = vacc.setdefault((a0, u), [None, None])
                for d in range(d0, d1):
                    q = qb[par][d, :, _lanes(u)]
                    for a in range(2):
                        t = kb[par][d, a0 + 8 * a:a0 + 8 * a + 8, :] * q
                        sums[a] = t if sums[a] is None else sums[a] + t
                if d1 == DH:
                    put(mxu_keys + a0, mxu_keys + a0 + 16, u, jnp.concatenate(sums, axis=0))

            def fetch(c, u):
                pend[c, u] = _unpack(probs[1 - par][_half(c * LANE, (c + 1) * LANE), _lanes(u)])

            def weigh(c, u):
                v_ref, o_ref = old
                o = _dot(v_ref[c // TPB, :, _lanes(c % TPB)], pend.pop((c, u)))
                acc[u] = acc[u] + o if c else o
                if c == NT - 1:
                    o_ref[u // TPB, :, _lanes(u % TPB)] = acc[u]

            def spread_k(d):
                r = d + 4 * (1 - par)
                kb[1 - par][d] = jnp.broadcast_to(nxt[0][r:r + 1, :], (LANE, kpad)).T[kpad - vpu_keys:]

            def spread_q(u):
                q = _unpack(nxt[1][u // TPB, :, _lanes(u % TPB)]).astype(F32)
                for d in range(DH):
                    r = d + 4 * (1 - par)
                    qb[1 - par][d, :, _lanes(u)] = jnp.broadcast_to(q[r:r + 1, :], (8, LANE))

            events = []
            for j in range(NT // group):
                t0 = j * NT * group
                cells = [(t0 + c * group + w, c, j * group + w) for c in range(NT) for w in range(group)]
                for t, c, u in cells if old is not None else []:
                    events.append((t - cfg["exlead"], 0, functools.partial(fetch, c, u)))
                    events.append((t, 1, functools.partial(weigh, c, u)))
                for t, c, u in cells if new is not None else []:
                    events.append((t - cfg["qlead"], 3, functools.partial(mxu_scores, c, u)))
                ds = cfg["dsplit"]
                parts = [(a0, j * group + (w + cfg["vrot"]) % group, DH * s // ds, DH * (s + 1) // ds)
                         for a0 in range(0, vpu_keys, 16) for w in range(group) for s in range(ds)]
                for n, part in enumerate(parts if new is not None and shared else []):
                    t = (t0 + NT * group * (n + 0.5) / len(parts)) * cfg["vspan"] / 100 + cfg["vstart"]
                    events.append((t, 2, functools.partial(vpu_scores, *part)))
            if nxt is not None:
                for job, count, a, b in ((spread_k, DH, cfg["bstart"], cfg["bspan"]),
                                         (spread_q, NT, cfg["qstart"], cfg["qspan"])):
                    for n in range(count):
                        events.append((NT * NT * (a + (b - a) * (n + 0.5) / count) / 100, 8, functools.partial(job, n)))
            events.sort(key=lambda e: e[:2])
            return [e[2] for e in events]

        def two_heads(j, carry):
            for par in (1, 0):
                h = 2 * j + 2 - par
                new, old, nxt = jnp.minimum(h, H - 1), h - 1, jnp.minimum(h + 1, H - 1)
                refs = (kw.at[new], qw.at[new]), (vw.at[old], oraw.at[old]), (kt.at[nxt], qw.at[nxt])

                @pl.when(h < H)
                def _():
                    for job in attention(*refs, par, cfg["gb"]):
                        job()
            return carry

        seen[0:2] = jnp.ones((2, 8, LANE), F32)
        seen[2] = jnp.zeros((8, LANE), F32)
        if cfg["only"] == 0:
            for job in attention((kw.at[0], qw.at[0]), None, (kt.at[1], qw.at[1]), 0, cfg["gb"]):
                job()
        lax.fori_loop(0, H // 2, two_heads, 0)
        if cfg["only"]:
            xv[0, 0:24, 0:RB] = oraw[0, 0].astype(BF16)
            return pltpu.sync_copy(xv.at[0], o_hbm.at[0:RB])

        def heads(i, u, h0, h1):
            row8 = lax.broadcasted_iota(I32, (8, LANE), 0)
            parts, sums = [], []
            for h in range(h0, h1, 2):
                e, o = oraw[h, i, :, _lanes(u)], oraw[h + 1, i, :, _lanes(u)]
                total = jnp.where(row8 < 4, o[0:8], e[16:24])
                inv = pl.reciprocal(total, approx=True)
                inv = inv * (2.0 - total * inv)
                parts += [e[0:16] * inv[4:5], jnp.where(row8 < 4, e[16:24], o[0:8]) * pltpu.roll(inv, 4, 0),
                          o[8:24] * inv[0:1]]
                sums.append(total)
            return jnp.concatenate(parts, axis=0), sums

        def gather_jobs(i, tiles):
            res, stats, n = {}, [], out_mm.rows // LANE

            def tile(u):
                h0 = tiles[0] * LANE // (2 * DH) * 2
                a, sums = heads(i, u, h0, min(H, (tiles[-1] + 1) * LANE // DH + 1))
                stats.append((functools.reduce(jnp.minimum, sums), functools.reduce(jnp.maximum, sums),
                              jnp.sum(a.reshape(-1, 8, LANE), axis=0)))
                for t in tiles:
                    res[u, t] = a[t * LANE - h0 * DH:(t + 1) * LANE - h0 * DH].T
                    att.at[i][_half(u * LANE, (u + 1) * LANE), _lanes(t)] = _pack(res[u, t])

            def operands(u, r):
                out_mm.put_input(lambda p, t: res[p * n + u, t][r:r + 32], att_op.at[i], u * LANE + r, u * LANE + r + 32)

            def record():
                lo, hi, total = zip(*stats)
                seen[0] = functools.reduce(jnp.minimum, lo, seen[0])
                seen[1] = functools.reduce(jnp.maximum, hi, seen[1])
                seen[2] = functools.reduce(jnp.add, total, seen[2])

            jobs = []
            for u in range(n):
                jobs += [functools.partial(tile, p * n + u) for p in range(out_mm.q)]
                if tiles[0] == 0:
                    jobs += [functools.partial(operands, u, r) for r in range(0, LANE, 32)]
            return jobs + [record]

        def mix(blocks, jobs, pending):
            spread = _Filler()
            spread.add(jobs, 0, out_mm.work * len(blocks) * 0.9)
            for i in blocks:
                filler = _Filler(spread)
                filler.add(gather_jobs(i, (4,)), 0, out_mm.rows * out_mm.kq * 5)
                if i == 0:
                    filler.add(pending, 0, out_mm.work * cfg["g2"] / 100)
                if i + 1 < NB:
                    filler.add(gather_jobs(i + 1, (0, 1, 2, 3)), 0, out_mm.work * cfg["g1"] / 100)
                for res in out_mm.columns(att.at[i], att_op.at[i], wo, wo_op, filler, 256):
                    for t, val in res.items():
                        hres[i, :, _lanes(t)] = xv[i, :, _lanes(t)].astype(F32) + val
                filler.flush()
            spread.flush()

        def project_heads(n, carry):
            @pl.when(n == 0)
            def _():
                last = attention(None, (vw.at[H - 1], oraw.at[H - 1]), None, H % 2, TPB)
                count = len(last) // NB + cfg["lh"]
                filler = _Filler()
                filler.add(gather_jobs(0, (0, 1, 2, 3)), 0, count)
                for job in last[:count]:
                    job()
                    filler.tick(1)
                filler.flush()
                mix(range(0, NB // 2), up_jobs[cut:], last[count:])

            @pl.when(n == 1)
            def _():
                mix(range(NB // 2, NB), norm_jobs(hres.at[0], 0, up_mm, hn_op, 16), [])
            return carry

        def feed_forward(i, carry):
            h_ref, next_ref, out_ref = hres.at[i], hres.at[jnp.minimum(i + 1, NB - 1)], xv.at[i]

            @pl.when(i != NB)
            def _():
                bias = b1[...].astype(F32).reshape(1, F)
                cols = {}
                for res in up_mm.columns(xn.at[0], hn_op.at[0], w1, w1_op, _Filler(), RB):
                    for t, val in res.items():
                        r = jnp.maximum(val + bias[:, _lanes(t)], 0.0)
                        cols[t] = r * r
                        act[:, _lanes(t)] = _pack(cols[t])
                    ready = [k for k in range(down_mm.kq) if k in cols and down_mm.kq + k in cols]
                    down_mm.put_input(lambda p, t: cols[t][p * down_mm.rows:(p + 1) * down_mm.rows],
                                      act_op.at[0], 0, down_mm.rows, ready)
                    for k in ready:
                        cols.pop(k)
                bias = b2[...].astype(F32).reshape(1, D)
                filler = _Filler()
                filler.add(norm_jobs(next_ref, 0, up_mm, hn_op, 16), 0, down_mm.work * 0.9)
                for res in down_mm.columns(act, act_op.at[0], w2, w2_op, filler, RB):
                    for t, val in res.items():
                        out_ref[:, _lanes(t)] = (h_ref[:, _lanes(t)] + (val + bias[:, _lanes(t)])).astype(BF16)
                        o_copy(i, t).start()
                filler.flush()
            return carry

        lax.fori_loop(0, 2, project_heads, 0)
        lax.fori_loop(0, NB, feed_forward, 0)
        safe = (seen[0] >= SUM_MIN) & (seen[1] <= SUM_MAX) & (jnp.abs(seen[2]) <= 3e38)
        unsafe = jnp.max(jnp.where(safe, cfg["force"], 1)) > 0
        for i in range(NB):
            for t in range(D // LANE):
                o_copy(i, t).wait()

        @pl.when(unsafe)
        def _():
            def head(n, carry):
                h, i = n // NB, n % NB
                q = _unpack(qw[h, i])

                def scores(c):
                    rows = pl.ds(pl.multiple_of(c * (LANE // 2), LANE // 2), LANE // 2)
                    return _dot(_unpack(kw[h, rows, :]), q)

                m = lax.fori_loop(0, NT, lambda c, m: jnp.maximum(m, jnp.max(scores(c), axis=0, keepdims=True)),
                                  jnp.full((1, RB), -jnp.inf, F32))

                def weigh(b, o):
                    for c in range(TPB):
                        o = o + _dot(vw[h, b, :, _lanes(c)], jnp.exp2(scores(b * TPB + c) - m))
                    return o
                oraw[h, i] = lax.fori_loop(0, NB, weigh, jnp.zeros((VR, RB), F32))
                return carry
            lax.fori_loop(0, H * NB, head, 0)

            def block(i, carry):
                x_copy(i).start()
                x_copy(i).wait()
                for u in range(TPB):
                    att.at[0][_half(u * LANE, (u + 1) * LANE), :] = _pack(heads(i, u, 0, H)[0].T)

                def rows(r, carry):
                    at = pl.ds(pl.multiple_of(r * 32, 32), 32)
                    a = _unpack(att[0, pl.ds(pl.multiple_of(r * 16, 16), 16), :])
                    hh = xv[i, at, :].astype(F32) + _dot(a, wo[...])
                    g = jnp.maximum(_dot(_ln(hh).astype(BF16), w1[...]) + b1[...].astype(F32).reshape(1, F), 0.0)
                    out = hh + (_dot((g * g).astype(BF16), w2[...]) + b2[...].astype(F32).reshape(1, D))
                    xv[i, at, :] = out.astype(BF16)
                    return carry
                lax.fori_loop(0, RB // 32, rows, 0)
                done = pltpu.make_async_copy(xv.at[i], o_hbm.at[pl.ds(i * RB, RB)], sem_x.at[i])
                done.start()
                done.wait()
                return carry
            lax.fori_loop(0, NB, block, 0)

    scratch = [
        pltpu.VMEM((NB, RB, D), BF16),
        pltpu.VMEM((D, 3 * D), BF16), pltpu.VMEM((D, D), BF16), pltpu.VMEM((D, F), BF16), pltpu.VMEM((F, D), BF16),
        qkv_mm.weight_scratch(), out_mm.weight_scratch(), up_mm.weight_scratch(), down_mm.weight_scratch(),
        pltpu.VMEM((2, RB // 2, D), I32), qkv_mm.input_scratch(2), up_mm.input_scratch(1),
        pltpu.VMEM((NB, RB // 2, D), I32), out_mm.input_scratch(NB),
        pltpu.VMEM((RB // 2, F), I32), down_mm.input_scratch(1),
        pltpu.VMEM((NB, RB, D), F32),
        pltpu.VMEM((H, S // 2, KD), I32), pltpu.VMEM((H, VR, kpad), F32),
        pltpu.VMEM((H, NB, KD // 2, RB), I32),
        pltpu.VMEM((H, NB, VR, RB), F32), pltpu.VMEM((H, NB, VR, RB), F32),
        pltpu.VMEM((4, 8, LANE), F32),
        pltpu.VMEM((S // 2, S), I32), pltpu.VMEM((S // 2, S), I32),
        pltpu.VMEM((DH, vpu_keys, LANE), F32), pltpu.VMEM((DH, vpu_keys, LANE), F32),
        pltpu.VMEM((DH, 8, S), F32), pltpu.VMEM((DH, 8, S), F32),
        pltpu.VMEM((F,), BF16), pltpu.VMEM((D,), BF16),
        pltpu.SemaphoreType.DMA((NB,)), pltpu.SemaphoreType.DMA((9,)), pltpu.SemaphoreType.DMA((NB * D // LANE,)),
    ]
    out = pl.pallas_call(
        kernel,
        out_shape=jax.ShapeDtypeStruct((S, D), BF16),
        in_specs=[pl.BlockSpec(memory_space=pl.ANY)] * 7,
        out_specs=pl.BlockSpec(memory_space=pl.ANY),
        scratch_shapes=scratch,
        compiler_params=pltpu.CompilerParams(
            vmem_limit_bytes=120 * 2**20, flags={"XLA_TPU_EVENLY_DISTRIBUTE_CRITICAL_NODES": True}),
    )(A_x.reshape(S, D), A_wqkv, A_wo, B_w1, B_b1, B_w2, B_b2)
    return out.reshape(1, S, D)


@jax.jit
def pallas_sequential_preLN__softmax_full_mha__dense_activation_squared_relu__prompt_kernel(
    A_x: jax.Array,
    A_wqkv: jax.Array,
    A_wo: jax.Array,
    B_x: jax.Array,
    B_w1: jax.Array,
    B_b1: jax.Array,
    B_w2: jax.Array,
    B_b2: jax.Array,
):
    del B_x
    return _run(CFG, A_x, A_wqkv, A_wo, B_w1, B_b1, B_w2, B_b2)
```

```python
import functools

import jax
import jax.numpy as jnp
from jax import lax
import jax.experimental.pallas as pl
import jax.experimental.pallas.tpu as pltpu

F32, BF16, I32 = jnp.float32, jnp.bfloat16, jnp.int32

S, D, F, H = 2048, 640, 1536, 32
DH = D // H
LANE = 128
NT = S // LANE
RB = 512
NB = S // RB
TPB = RB // LANE
KD = 32
VR = 24
EPS = 1e-5
QSCALE = float(DH ** -0.5 * 1.4426950408889634)
SUM_MIN, SUM_MAX = 2.0 ** -40, 2.0 ** 100

VPU_KEYS = 272
KPAD = 384
QKV_STAGES = (0, 2, 4, 7)

_A_TERMS = (((1, 0), (1, 3)), ((1, 3),), ((1, 0), (1, 1)), ((1, 1), (-1, 3)), ((1, 2), (1, 3)), ((1, 0),), ((1, 2), (-1, 0)))
_B_TERMS = (((1, 0), (1, 3)), ((1, 2), (-1, 0)), ((1, 3),), ((1, 2), (1, 3)), ((1, 0),), ((1, 1), (-1, 3)), ((1, 0), (1, 1)))
_C_TERMS = (((1, 0), (1, 3)), ((1, 0), (1, 2)), ((-1, 0), (1, 1)), ((1, 0),), ((1, 2), (-1, 3)), ((1, 1), (1, 3)), ((1, 3),))


def _ln(x):
    mean = jnp.mean(x, axis=-1, keepdims=True)
    xc = x - mean
    var = jnp.mean(xc * xc, axis=-1, keepdims=True)
    return xc * lax.rsqrt(var + EPS)


def _dot(a, b):
    return jnp.dot(a, b, preferred_element_type=F32)


def _lanes(u):
    return slice(u * LANE, (u + 1) * LANE)


def _pack(v):
    return pltpu.bitcast(v.astype(BF16), I32)


def _unpack(v):
    return pltpu.bitcast(v, BF16)


def _half(a, b):
    return slice(a // 2, b // 2)


def _operands(blocks, terms, level):
    if level == 0:
        return [blocks[0][0]]
    n = len(blocks) // 2
    out = []
    for (_, first), *rest in terms:
        def combine(i, j):
            val = blocks[first // 2 * n + i][first % 2 * n + j]
            for sign, q in rest:
                other = blocks[q // 2 * n + i][q % 2 * n + j]
                val = val + other if sign > 0 else val - other
            return val
        out += _operands([[combine(i, j) for j in range(n)] for i in range(n)], terms, level - 1)
    return out


def _combine(product):
    out = {}
    for r, term in enumerate(_C_TERMS):
        grid = product(r)
        n = len(grid)
        for sign, q in term:
            for i in range(n):
                for j in range(n):
                    key = (q // 2 * n + i, q % 2 * n + j)
                    if key not in out:
                        out[key] = grid[i][j]
                    else:
                        out[key] = out[key] + grid[i][j] if sign > 0 else out[key] - grid[i][j]
    return [[out[i, j] for j in range(2 * n)] for i in range(2 * n)]


class _Filler:
    def __init__(self, parent=None):
        self.jobs, self.now, self.parent = [], 0, parent

    def add(self, jobs, start, stop):
        self.jobs += [(start + (stop - start) * (n + 0.5) / len(jobs), job) for n, job in enumerate(jobs)]
        self.jobs.sort(key=lambda e: e[0])

    def tick(self, work):
        self.now += work
        if self.parent is not None:
            self.parent.tick(work)
        while self.jobs and self.jobs[0][0] <= self.now:
            self.jobs.pop(0)[1]()

    def flush(self):
        while self.jobs:
            self.jobs.pop(0)[1]()


class _Linear:
    def __init__(self, k, n, level):
        self.k, self.n, self.level, self.q = k, n, level, 2 ** level
        self.kq = k // (LANE * self.q)
        self.nq = n // (LANE * self.q)
        self.rows = RB // self.q
        self.work = (7 ** level * self.rows * self.kq * self.nq
                     + RB * ((k // LANE) * (n // LANE) - self.kq * self.nq * self.q ** 2))

    def weight_scratch(self):
        return pltpu.VMEM((7 ** self.level, self.kq * LANE // 2, self.nq * LANE), I32)

    def input_scratch(self, slots):
        return pltpu.VMEM((slots, 7 ** self.level, self.rows // 2, self.kq * LANE), I32)

    def weight_jobs(self, w_ref, op_ref, groups=None):
        part = self.kq * LANE

        def job(r0, j):
            blocks = [[w_ref[a * part + r0:a * part + r0 + 16, _lanes(b * self.nq + j)].astype(F32)
                       for b in range(self.q)] for a in range(self.q)]
            for r, op in enumerate(_operands(blocks, _B_TERMS, self.level)):
                op_ref.at[r][_half(r0, r0 + 16), _lanes(j)] = _pack(op)
        return [functools.partial(job, r0, j) for j in (range(self.nq) if groups is None else groups)
                for r0 in range(0, part, 16)]

    def put_input(self, block, op_ref, r0, r1, tiles=None):
        for kt in range(self.kq) if tiles is None else tiles:
            blocks = [[block(i, b * self.kq + kt) for b in range(self.q)] for i in range(self.q)]
            for r, op in enumerate(_operands(blocks, _A_TERMS, self.level)):
                op_ref.at[r][_half(r0, r1), _lanes(kt)] = _pack(op)

    def columns(self, a_ref, aop_ref, w_ref, wop_ref, filler, step):
        def dot(a, b):
            out = _dot(a, b)
            filler.tick(a.shape[0] * a.shape[1] // LANE)
            return out

        def direct(t, k0):
            return jnp.concatenate([dot(_unpack(a_ref[_half(m, m + step), k0:self.k]), w_ref[k0:self.k, _lanes(t)])
                                    for m in range(0, RB, step)], axis=0)

        k0 = self.kq * self.q * LANE
        for j in range(self.nq):
            def product(r):
                return [[dot(_unpack(aop_ref[r]), _unpack(wop_ref[r, :, _lanes(j)]))]]
            if self.level == 1:
                grid = _combine(product)
            else:
                grid = _combine(lambda r: _combine(lambda s: product(7 * r + s)))
            out = {}
            for b in range(self.q):
                t = b * self.nq + j
                out[t] = jnp.concatenate([row[b] for row in grid], axis=0)
                if k0 < self.k:
                    out[t] = out[t] + direct(t, k0)
            yield out
        for t in range(self.nq * self.q, self.n // LANE):
            yield {t: direct(t, 0)}


@jax.jit
def pallas_sequential_preLN__softmax_full_mha__dense_activation_squared_relu__prompt_kernel(
    A_x: jax.Array,
    A_wqkv: jax.Array,
    A_wo: jax.Array,
    B_x: jax.Array,
    B_w1: jax.Array,
    B_b1: jax.Array,
    B_w2: jax.Array,
    B_b2: jax.Array,
):
    del B_x
    mxu_keys = S - VPU_KEYS
    qkv_mm, out_mm = _Linear(D, 3 * D, 1), _Linear(D, D, 1)
    up_mm, down_mm = _Linear(D, F, 2), _Linear(F, D, 1)

    def kernel(x_hbm, wqkv_hbm, wo_hbm, w1_hbm, b1_hbm, w2_hbm, b2_hbm, o_hbm,
               xv, wqkv, wo, w1, w2, wqkv_op, wo_op, w1_op, w2_op, xn, xn_op, hn_op, att, att_op, act, act_op,
               hres, kw, kt, qw, vw, oraw, seen, p0, p1, kb0, kb1, qb0, qb1, b1, b2, sem_x, sem_w, sem_o):
        probs, kb, qb = (p0, p1), (kb0, kb1), (qb0, qb1)

        def x_copy(i):
            return pltpu.make_async_copy(x_hbm.at[pl.ds(i * RB, RB)], xv.at[i], sem_x.at[i])

        def o_copy(i, t):
            return pltpu.make_async_copy(xv.at[i, :, _lanes(t)], o_hbm.at[pl.ds(i * RB, RB), _lanes(t)],
                                         sem_o.at[i * (D // LANE) + t])

        half = qkv_mm.nq * LANE
        spans = [(side + a * LANE, side + b * LANE if b < qkv_mm.nq or not side else 3 * D)
                 for a, b in zip(QKV_STAGES, QKV_STAGES[1:]) for side in (0, half)]
        pairs = [(wqkv_hbm.at[:, a:b], wqkv.at[:, a:b]) for a, b in spans]
        pairs += [(wo_hbm, wo), (w1_hbm, w1), (w2_hbm, w2), (b1_hbm, b1), (b2_hbm, b2)]
        w_copies = [pltpu.make_async_copy(src, dst, sem_w.at[n]) for n, (src, dst) in enumerate(pairs)]
        qkv_copies, other_copies = w_copies[:len(spans)], w_copies[len(spans):]

        def qkv_stage(n):
            qkv_copies[2 * n].wait()
            qkv_copies[2 * n + 1].wait()
            if n + 2 == len(QKV_STAGES):
                x_copy(1).wait()
                for i in range(2, NB):
                    x_copy(i).start()
            for job in qkv_mm.weight_jobs(wqkv, wqkv_op, range(QKV_STAGES[n], QKV_STAGES[n + 1])):
                job()

        def norm_jobs(src_ref, slot, mm, op_ref, step):
            def job(r):
                ys = []
                for i in range(mm.q):
                    a = i * mm.rows + r
                    ys.append(_ln(src_ref[a:a + step, :].astype(F32)))
                    xn.at[slot][_half(a, a + step), :] = _pack(ys[i])
                mm.put_input(lambda i, t: ys[i][:, _lanes(t)], op_ref.at[slot], r, r + step)
            return [functools.partial(job, r) for r in range(0, mm.rows, step)]

        def project(i, jobs, step):
            filler = _Filler()
            for part in jobs:
                if i > 0:
                    filler.add(part, 0, qkv_mm.work * 0.98)
                else:
                    filler.add(part, qkv_mm.work * (QKV_STAGES[-2] + 0.1) / qkv_mm.nq, qkv_mm.work * 0.94)
            row = lax.broadcasted_iota(I32, (KD, RB), 0)
            row8 = lax.broadcasted_iota(I32, (8, RB), 0)
            nd = D // LANE
            tiles, todo = {}, [(part, h) for part in range(3) for h in range(H)]

            def window(part, start, size, axis):
                pieces = []
                for t in range(start // LANE, (min(start + size, D) - 1) // LANE + 1):
                    a, b = max(start - t * LANE, 0), min(start + size - t * LANE, LANE)
                    pieces.append(lax.slice_in_dim(tiles[part, t], a, b, axis=axis))
                if start + size > D:
                    pieces.append(jnp.zeros_like(lax.slice_in_dim(pieces[0], 0, start + size - D, axis=axis)))
                return pieces[0] if len(pieces) == 1 else jnp.concatenate(pieces, axis=axis)

            for n, res in enumerate(qkv_mm.columns(xn.at[i % 2], xn_op.at[i % 2], wqkv, wqkv_op, filler, step)):
                if i == 0 and n + 1 in QKV_STAGES[1:-1]:
                    qkv_stage(QKV_STAGES.index(n + 1))
                for t, val in res.items():
                    if t // nd == 0:
                        tiles[0, t % nd] = (val * QSCALE).T
                    elif t // nd == 1:
                        tiles[1, t % nd] = _pack(val)
                        if i == NB - 1:
                            tiles[3, t % nd] = val[RB - KPAD:].T
                    else:
                        tiles[2, t % nd] = val.T
                for part, h in list(todo):
                    b0 = 8 * (DH * h // 8)
                    if (part, b0 // LANE) not in tiles or (part, (min(b0 + KD, D) - 1) // LANE) not in tiles:
                        continue
                    todo.remove((part, h))
                    if part == 0:
                        lo = DH * h - b0
                        qw.at[h, i][...] = _pack(jnp.where((row >= lo) & (row < lo + DH), window(0, b0, KD, 0), 0.0))
                    elif part == 1:
                        kw[h, _half(i * RB, (i + 1) * RB), :] = window(1, b0, KD, 1)
                        if i == NB - 1:
                            kt[h] = window(3, b0, VR, 0)
                    elif h % 2 == 0:
                        vw[h, i, 0:16] = window(2, b0, 16, 0)
                        vw[h, i, 16:24] = jnp.where(row8 < 4, window(2, b0 + 16, 8, 0), 1.0)
                    else:
                        vw[h, i, 0:8] = jnp.where(row8 < 4, 1.0, window(2, b0, 8, 0))
                        vw[h, i, 8:24] = window(2, b0 + 8, 16, 0)
            assert not todo
            filler.flush()

        def first_blocks(n, carry):
            @pl.when(n == 0)
            def _():
                project(0, [norm_jobs(xv.at[1], 1, qkv_mm, xn_op, 32)], 256)

            @pl.when(n < 1)
            def _():
                for i in range(2, NB):
                    x_copy(i).wait()
                for c in other_copies:
                    c.start()

            @pl.when(n != 1)
            def _():
                for i in range(1, NB - 1):
                    project(i, [norm_jobs(xv.at[i + 1], (i + 1) % 2, qkv_mm, xn_op, 16)], 128)

            @pl.when(n + 1 == 1)
            def _():
                for c in other_copies:
                    c.wait()
            return carry

        x_copy(0).start()
        for c in qkv_copies[:2]:
            c.start()
        x_copy(0).wait()
        for c in qkv_copies[2:]:
            c.start()
        x_copy(1).start()
        for job in norm_jobs(xv.at[0], 0, qkv_mm, xn_op, 64):
            job()
        qkv_stage(0)
        lax.fori_loop(0, 2, first_blocks, 0)
        project(NB - 1, [out_mm.weight_jobs(wo, wo_op), down_mm.weight_jobs(w2, w2_op),
                         up_mm.weight_jobs(w1, w1_op)], 128)

        def attention(new, old, nxt, par, group):
            acc, pend, vacc = {}, {}, {}
            shared = old is not None
            bounds = [16 * ((mxu_keys if shared else S) // 16 * c // NT) for c in range(NT + 1)]

            def put(a, b, u, s):
                probs[par][_half(a, b), _lanes(u)] = _pack(jnp.exp2(s))

            def mxu_scores(c, u):
                k_ref, q_ref = new
                a, b = bounds[c], bounds[c + 1]
                put(a, b, u, _dot(_unpack(k_ref[_half(a, b), :]), _unpack(q_ref[u // TPB, :, _lanes(u % TPB)])))

            def vpu_scores(a0, u, d0, d1):
                sums = vacc.setdefault((a0, u), [None, None])
                for d in range(d0, d1):
                    q = qb[par][d, :, _lanes(u)]
                    for a in range(2):
                        t = kb[par][d, a0 + 8 * a:a0 + 8 * a + 8, :] * q
                        sums[a] = t if sums[a] is None else sums[a] + t
                if d1 == DH:
                    put(mxu_keys + a0, mxu_keys + a0 + 16, u, jnp.concatenate(sums, axis=0))

            def fetch(c, u):
                pend[c, u] = _unpack(probs[1 - par][_half(c * LANE, (c + 1) * LANE), _lanes(u)])

            def weigh(c, u):
                v_ref, o_ref = old
                o = _dot(v_ref[c // TPB, :, _lanes(c % TPB)], pend.pop((c, u)))
                acc[u] = acc[u] + o if c else o
                if c == NT - 1:
                    o_ref[u // TPB, :, _lanes(u % TPB)] = acc[u]

            def spread_k(d):
                r = d + 4 * (1 - par)
                kb[1 - par][d] = jnp.broadcast_to(nxt[0][r:r + 1, :], (LANE, KPAD)).T[KPAD - VPU_KEYS:]

            def spread_q(u):
                q = _unpack(nxt[1][u // TPB, :, _lanes(u % TPB)]).astype(F32)
                for d in range(DH):
                    r = d + 4 * (1 - par)
                    qb[1 - par][d, :, _lanes(u)] = jnp.broadcast_to(q[r:r + 1, :], (8, LANE))

            events = []
            for j in range(NT // group):
                t0 = j * NT * group
                cells = [(t0 + c * group + w, c, j * group + w) for c in range(NT) for w in range(group)]
                for t, c, u in cells if old is not None else []:
                    events.append((t - 4, 0, functools.partial(fetch, c, u)))
                    events.append((t, 1, functools.partial(weigh, c, u)))
                for t, c, u in cells if new is not None else []:
                    events.append((t - 3.5, 3, functools.partial(mxu_scores, c, u)))
                parts = [(a0, j * group + w, d, d + 2)
                         for a0 in range(0, VPU_KEYS, 16) for w in range(group) for d in range(0, DH, 2)]
                for n, part in enumerate(parts if new is not None and shared else []):
                    t = (t0 + NT * group * (n + 0.5) / len(parts)) * 99.0 / 100 + 3.0
                    events.append((t, 2, functools.partial(vpu_scores, *part)))
            if nxt is not None:
                for job, count, a, b in ((spread_k, DH, 20, 80), (spread_q, NT, 30, 80)):
                    for n in range(count):
                        events.append((NT * NT * (a + (b - a) * (n + 0.5) / count) / 100, 8, functools.partial(job, n)))
            events.sort(key=lambda e: e[:2])
            return [e[2] for e in events]

        def two_heads(j, carry):
            for par in (1, 0):
                h = 2 * j + 2 - par
                new, old, nxt = jnp.minimum(h, H - 1), h - 1, jnp.minimum(h + 1, H - 1)
                refs = (kw.at[new], qw.at[new]), (vw.at[old], oraw.at[old]), (kt.at[nxt], qw.at[nxt])

                @pl.when(h < H)
                def _():
                    for job in attention(*refs, par, NT):
                        job()
            return carry

        seen[0:2] = jnp.ones((2, 8, LANE), F32)
        seen[2] = jnp.zeros((8, LANE), F32)
        for job in attention((kw.at[0], qw.at[0]), None, (kt.at[1], qw.at[1]), 0, NT):
            job()
        lax.fori_loop(0, H // 2, two_heads, 0)

        def heads(i, u, h0, h1):
            row8 = lax.broadcasted_iota(I32, (8, LANE), 0)
            parts, sums = [], []
            for h in range(h0, h1, 2):
                e, o = oraw[h, i, :, _lanes(u)], oraw[h + 1, i, :, _lanes(u)]
                total = jnp.where(row8 < 4, o[0:8], e[16:24])
                inv = pl.reciprocal(total, approx=True)
                inv = inv * (2.0 - total * inv)
                parts += [e[0:16] * inv[4:5], jnp.where(row8 < 4, e[16:24], o[0:8]) * pltpu.roll(inv, 4, 0),
                          o[8:24] * inv[0:1]]
                sums.append(total)
            return jnp.concatenate(parts, axis=0), sums

        def gather_jobs(i, tiles):
            res, stats, n = {}, [], out_mm.rows // LANE

            def tile(u):
                h0 = tiles[0] * LANE // (2 * DH) * 2
                a, sums = heads(i, u, h0, min(H, (tiles[-1] + 1) * LANE // DH + 1))
                stats.append((functools.reduce(jnp.minimum, sums), functools.reduce(jnp.maximum, sums),
                              jnp.sum(a.reshape(-1, 8, LANE), axis=0)))
                for t in tiles:
                    res[u, t] = a[t * LANE - h0 * DH:(t + 1) * LANE - h0 * DH].T
                    att.at[i][_half(u * LANE, (u + 1) * LANE), _lanes(t)] = _pack(res[u, t])

            def operands(u, r):
                out_mm.put_input(lambda p, t: res[p * n + u, t][r:r + 32], att_op.at[i], u * LANE + r, u * LANE + r + 32)

            def record():
                lo, hi, total = zip(*stats)
                seen[0] = functools.reduce(jnp.minimum, lo, seen[0])
                seen[1] = functools.reduce(jnp.maximum, hi, seen[1])
                seen[2] = functools.reduce(jnp.add, total, seen[2])

            jobs = []
            for u in range(n):
                jobs += [functools.partial(tile, p * n + u) for p in range(out_mm.q)]
                if tiles[0] == 0:
                    jobs += [functools.partial(operands, u, r) for r in range(0, LANE, 32)]
            return jobs + [record]

        def mix(blocks, jobs, pending):
            spread = _Filler()
            spread.add(jobs, 0, out_mm.work * len(blocks) * 0.9)
            for i in blocks:
                filler = _Filler(spread)
                filler.add(gather_jobs(i, (4,)), 0, out_mm.rows * out_mm.kq * 5)
                if i == 0:
                    filler.add(pending, 0, out_mm.work * 0.95)
                if i + 1 < NB:
                    filler.add(gather_jobs(i + 1, (0, 1, 2, 3)), 0, out_mm.work * 0.85)
                for res in out_mm.columns(att.at[i], att_op.at[i], wo, wo_op, filler, 256):
                    for t, val in res.items():
                        hres[i, :, _lanes(t)] = xv[i, :, _lanes(t)].astype(F32) + val
                filler.flush()
            spread.flush()

        def project_heads(n, carry):
            @pl.when(n == 0)
            def _():
                last = attention(None, (vw.at[H - 1], oraw.at[H - 1]), None, H % 2, TPB)
                count = len(last) // NB + 8
                filler = _Filler()
                filler.add(gather_jobs(0, (0, 1, 2, 3)), 0, count)
                for job in last[:count]:
                    job()
                    filler.tick(1)
                filler.flush()
                mix(range(0, NB // 2), [], last[count:])

            @pl.when(n == 1)
            def _():
                mix(range(NB // 2, NB), norm_jobs(hres.at[0], 0, up_mm, hn_op, 16), [])
            return carry

        def feed_forward(i, carry):
            h_ref, next_ref, out_ref = hres.at[i], hres.at[jnp.minimum(i + 1, NB - 1)], xv.at[i]

            @pl.when(i != NB)
            def _():
                bias = b1[...].astype(F32).reshape(1, F)
                cols = {}
                for res in up_mm.columns(xn.at[0], hn_op.at[0], w1, w1_op, _Filler(), RB):
                    for t, val in res.items():
                        r = jnp.maximum(val + bias[:, _lanes(t)], 0.0)
                        cols[t] = r * r
                        act[:, _lanes(t)] = _pack(cols[t])
                    ready = [k for k in range(down_mm.kq) if k in cols and down_mm.kq + k in cols]
                    down_mm.put_input(lambda p, t: cols[t][p * down_mm.rows:(p + 1) * down_mm.rows],
                                      act_op.at[0], 0, down_mm.rows, ready)
                    for k in ready:
                        cols.pop(k)
                bias = b2[...].astype(F32).reshape(1, D)
                filler = _Filler()
                filler.add(norm_jobs(next_ref, 0, up_mm, hn_op, 16), 0, down_mm.work * 0.9)
                for res in down_mm.columns(act, act_op.at[0], w2, w2_op, filler, RB):
                    for t, val in res.items():
                        out_ref[:, _lanes(t)] = (h_ref[:, _lanes(t)] + (val + bias[:, _lanes(t)])).astype(BF16)
                        o_copy(i, t).start()
                filler.flush()
            return carry

        lax.fori_loop(0, 2, project_heads, 0)
        lax.fori_loop(0, NB, feed_forward, 0)
        safe = (seen[0] >= SUM_MIN) & (seen[1] <= SUM_MAX) & (jnp.abs(seen[2]) <= 3e38)
        unsafe = jnp.max(jnp.where(safe, 0, 1)) > 0
        for i in range(NB):
            for t in range(D // LANE):
                o_copy(i, t).wait()

        @pl.when(unsafe)
        def _():
            def head(n, carry):
                h, i = n // NB, n % NB
                q = _unpack(qw[h, i])

                def scores(c):
                    rows = pl.ds(pl.multiple_of(c * (LANE // 2), LANE // 2), LANE // 2)
                    return _dot(_unpack(kw[h, rows, :]), q)

                m = lax.fori_loop(0, NT, lambda c, m: jnp.maximum(m, jnp.max(scores(c), axis=0, keepdims=True)),
                                  jnp.full((1, RB), -jnp.inf, F32))

                def weigh(b, o):
                    for c in range(TPB):
                        o = o + _dot(vw[h, b, :, _lanes(c)], jnp.exp2(scores(b * TPB + c) - m))
                    return o
                oraw[h, i] = lax.fori_loop(0, NB, weigh, jnp.zeros((VR, RB), F32))
                return carry
            lax.fori_loop(0, H * NB, head, 0)

            def block(i, carry):
                x_copy(i).start()
                x_copy(i).wait()
                for u in range(TPB):
                    att.at[0][_half(u * LANE, (u + 1) * LANE), :] = _pack(heads(i, u, 0, H)[0].T)

                def rows(r, carry):
                    at = pl.ds(pl.multiple_of(r * 32, 32), 32)
                    a = _unpack(att[0, pl.ds(pl.multiple_of(r * 16, 16), 16), :])
                    hh = xv[i, at, :].astype(F32) + _dot(a, wo[...])
                    g = jnp.maximum(_dot(_ln(hh).astype(BF16), w1[...]) + b1[...].astype(F32).reshape(1, F), 0.0)
                    out = hh + (_dot((g * g).astype(BF16), w2[...]) + b2[...].astype(F32).reshape(1, D))
                    xv[i, at, :] = out.astype(BF16)
                    return carry
                lax.fori_loop(0, RB // 32, rows, 0)
                done = pltpu.make_async_copy(xv.at[i], o_hbm.at[pl.ds(i * RB, RB)], sem_x.at[i])
                done.start()
                done.wait()
                return carry
            lax.fori_loop(0, NB, block, 0)

    scratch = [
        pltpu.VMEM((NB, RB, D), BF16),
        pltpu.VMEM((D, 3 * D), BF16), pltpu.VMEM((D, D), BF16), pltpu.VMEM((D, F), BF16), pltpu.VMEM((F, D), BF16),
        qkv_mm.weight_scratch(), out_mm.weight_scratch(), up_mm.weight_scratch(), down_mm.weight_scratch(),
        pltpu.VMEM((2, RB // 2, D), I32), qkv_mm.input_scratch(2), up_mm.input_scratch(1),
        pltpu.VMEM((NB, RB // 2, D), I32), out_mm.input_scratch(NB),
        pltpu.VMEM((RB // 2, F), I32), down_mm.input_scratch(1),
        pltpu.VMEM((NB, RB, D), F32),
        pltpu.VMEM((H, S // 2, KD), I32), pltpu.VMEM((H, VR, KPAD), F32),
        pltpu.VMEM((H, NB, KD // 2, RB), I32),
        pltpu.VMEM((H, NB, VR, RB), F32), pltpu.VMEM((H, NB, VR, RB), F32),
        pltpu.VMEM((4, 8, LANE), F32),
        pltpu.VMEM((S // 2, S), I32), pltpu.VMEM((S // 2, S), I32),
        pltpu.VMEM((DH, VPU_KEYS, LANE), F32), pltpu.VMEM((DH, VPU_KEYS, LANE), F32),
        pltpu.VMEM((DH, 8, S), F32), pltpu.VMEM((DH, 8, S), F32),
        pltpu.VMEM((F,), BF16), pltpu.VMEM((D,), BF16),
        pltpu.SemaphoreType.DMA((NB,)), pltpu.SemaphoreType.DMA((2 * len(QKV_STAGES) + 3,)), pltpu.SemaphoreType.DMA((NB * D // LANE,)),
    ]
    out = pl.pallas_call(
        kernel,
        out_shape=jax.ShapeDtypeStruct((S, D), BF16),
        in_specs=[pl.BlockSpec(memory_space=pl.ANY)] * 7,
        out_specs=pl.BlockSpec(memory_space=pl.ANY),
        scratch_shapes=scratch,
        compiler_params=pltpu.CompilerParams(
            vmem_limit_bytes=120 * 2**20, flags={"XLA_TPU_EVENLY_DISTRIBUTE_CRITICAL_NODES": True}),
    )(A_x.reshape(S, D), A_wqkv, A_wo, B_w1, B_b1, B_w2, B_b2)
    return out.reshape(1, S, D)
```

```python
import functools

import jax
import jax.numpy as jnp
from jax import lax
import jax.experimental.pallas as pl
import jax.experimental.pallas.tpu as pltpu

F32, BF16, I32 = jnp.float32, jnp.bfloat16, jnp.int32

S, D, F, H = 2048, 640, 1536, 32
DH = D // H
LANE = 128
NT = S // LANE
RB = 512
NB = S // RB
TPB = RB // LANE
KD = 32
VR = 24
EPS = 1e-5
QSCALE = float(DH ** -0.5 * 1.4426950408889634)
SUM_MIN, SUM_MAX = 2.0 ** -40, 2.0 ** 100

VPU_KEYS = 272
KPAD = 384
QKV_STAGES = (0, 2, 4, 7)

_A_TERMS = (((1, 0), (1, 3)), ((1, 3),), ((1, 0), (1, 1)), ((1, 1), (-1, 3)), ((1, 2), (1, 3)), ((1, 0),), ((1, 2), (-1, 0)))
_B_TERMS = (((1, 0), (1, 3)), ((1, 2), (-1, 0)), ((1, 3),), ((1, 2), (1, 3)), ((1, 0),), ((1, 1), (-1, 3)), ((1, 0), (1, 1)))
_C_TERMS = (((1, 0), (1, 3)), ((1, 0), (1, 2)), ((-1, 0), (1, 1)), ((1, 0),), ((1, 2), (-1, 3)), ((1, 1), (1, 3)), ((1, 3),))


def _ln(x):
    mean = jnp.mean(x, axis=-1, keepdims=True)
    xc = x - mean
    var = jnp.mean(xc * xc, axis=-1, keepdims=True)
    return xc * lax.rsqrt(var + EPS)


def _dot(a, b):
    return jnp.dot(a, b, preferred_element_type=F32)


def _lanes(u):
    return slice(u * LANE, (u + 1) * LANE)


def _pack(v):
    return pltpu.bitcast(v.astype(BF16), I32)


def _unpack(v):
    return pltpu.bitcast(v, BF16)


def _half(a, b):
    return slice(a // 2, b // 2)


def _operands(blocks, terms, level):
    if level == 0:
        return [blocks[0][0]]
    n = len(blocks) // 2
    out = []
    for (_, first), *rest in terms:
        def combine(i, j):
            val = blocks[first // 2 * n + i][first % 2 * n + j]
            for sign, q in rest:
                other = blocks[q // 2 * n + i][q % 2 * n + j]
                val = val + other if sign > 0 else val - other
            return val
        out += _operands([[combine(i, j) for j in range(n)] for i in range(n)], terms, level - 1)
    return out


def _combine(product):
    out = {}
    for r, term in enumerate(_C_TERMS):
        grid = product(r)
        n = len(grid)
        for sign, q in term:
            for i in range(n):
                for j in range(n):
                    key = (q // 2 * n + i, q % 2 * n + j)
                    if key not in out:
                        out[key] = grid[i][j]
                    else:
                        out[key] = out[key] + grid[i][j] if sign > 0 else out[key] - grid[i][j]
    return [[out[i, j] for j in range(2 * n)] for i in range(2 * n)]


class _Filler:
    def __init__(self, parent=None):
        self.jobs, self.now, self.parent = [], 0, parent

    def add(self, jobs, start, stop):
        self.jobs += [(start + (stop - start) * (n + 0.5) / len(jobs), job) for n, job in enumerate(jobs)]
        self.jobs.sort(key=lambda e: e[0])

    def tick(self, work):
        self.now += work
        if self.parent is not None:
            self.parent.tick(work)
        while self.jobs and self.jobs[0][0] <= self.now:
            self.jobs.pop(0)[1]()

    def flush(self):
        while self.jobs:
            self.jobs.pop(0)[1]()


class _Linear:
    def __init__(self, k, n, level):
        self.k, self.n, self.level, self.q = k, n, level, 2 ** level
        self.kq = k // (LANE * self.q)
        self.nq = n // (LANE * self.q)
        self.rows = RB // self.q
        self.work = (7 ** level * self.rows * self.kq * self.nq
                     + RB * ((k // LANE) * (n // LANE) - self.kq * self.nq * self.q ** 2))

    def weight_scratch(self):
        return pltpu.VMEM((7 ** self.level, self.kq * LANE // 2, self.nq * LANE), I32)

    def input_scratch(self, slots):
        return pltpu.VMEM((slots, 7 ** self.level, self.rows // 2, self.kq * LANE), I32)

    def weight_jobs(self, w_ref, op_ref, groups=None):
        part = self.kq * LANE

        def job(r0, j):
            blocks = [[w_ref[a * part + r0:a * part + r0 + 16, _lanes(b * self.nq + j)].astype(F32)
                       for b in range(self.q)] for a in range(self.q)]
            for r, op in enumerate(_operands(blocks, _B_TERMS, self.level)):
                op_ref.at[r][_half(r0, r0 + 16), _lanes(j)] = _pack(op)
        return [functools.partial(job, r0, j) for j in (range(self.nq) if groups is None else groups)
                for r0 in range(0, part, 16)]

    def put_input(self, block, op_ref, r0, r1, tiles=None):
        for kt in range(self.kq) if tiles is None else tiles:
            blocks = [[block(i, b * self.kq + kt) for b in range(self.q)] for i in range(self.q)]
            for r, op in enumerate(_operands(blocks, _A_TERMS, self.level)):
                op_ref.at[r][_half(r0, r1), _lanes(kt)] = _pack(op)

    def columns(self, a_ref, aop_ref, w_ref, wop_ref, filler, step, rest_first=False):
        def dot(a, b):
            out = _dot(a, b)
            filler.tick(a.shape[0] * a.shape[1] // LANE)
            return out

        def direct(t, k0):
            return jnp.concatenate([dot(_unpack(a_ref[_half(m, m + step), k0:self.k]), w_ref[k0:self.k, _lanes(t)])
                                    for m in range(0, RB, step)], axis=0)

        k0 = self.kq * self.q * LANE
        for j in range(self.nq):
            tiles = [b * self.nq + j for b in range(self.q)]
            rest = {t: direct(t, k0) for t in tiles if rest_first}

            def product(r):
                return [[dot(_unpack(aop_ref[r]), _unpack(wop_ref[r, :, _lanes(j)]))]]
            if self.level == 1:
                grid = _combine(product)
            else:
                grid = _combine(lambda r: _combine(lambda s: product(7 * r + s)))
            out = {}
            for b, t in enumerate(tiles):
                out[t] = jnp.concatenate([row[b] for row in grid], axis=0)
                if k0 < self.k:
                    out[t] = out[t] + (rest[t] if rest_first else direct(t, k0))
            yield out
        for t in range(self.nq * self.q, self.n // LANE):
            yield {t: direct(t, 0)}


@jax.jit
def pallas_sequential_preLN__softmax_full_mha__dense_activation_squared_relu__prompt_kernel(
    A_x: jax.Array,
    A_wqkv: jax.Array,
    A_wo: jax.Array,
    B_x: jax.Array,
    B_w1: jax.Array,
    B_b1: jax.Array,
    B_w2: jax.Array,
    B_b2: jax.Array,
):
    del B_x
    mxu_keys = S - VPU_KEYS
    qkv_mm, out_mm = _Linear(D, 3 * D, 1), _Linear(D, D, 1)
    up_mm, down_mm = _Linear(D, F, 2), _Linear(F, D, 1)

    def kernel(x_hbm, wqkv_hbm, wo_hbm, w1_hbm, b1_hbm, w2_hbm, b2_hbm, o_hbm,
               xv, wqkv, wo, w1, w2, wqkv_op, wo_op, w1_op, w2_op, xn, xn_op, hn_op, att, att_op, act, act_op,
               hres, kw, kt, qw, vw, oraw, seen, p0, p1, kb0, kb1, qb0, qb1, b1, b2, sem_x, sem_w, sem_o):
        probs, kb, qb = (p0, p1), (kb0, kb1), (qb0, qb1)

        def x_copy(i):
            return pltpu.make_async_copy(x_hbm.at[pl.ds(i * RB, RB)], xv.at[i], sem_x.at[i])

        def o_copy(i, t):
            return pltpu.make_async_copy(xv.at[i, :, _lanes(t)], o_hbm.at[pl.ds(i * RB, RB), _lanes(t)],
                                         sem_o.at[i * (D // LANE) + t])

        half = qkv_mm.nq * LANE
        spans = [(side + a * LANE, side + b * LANE if b < qkv_mm.nq or not side else 3 * D)
                 for a, b in zip(QKV_STAGES, QKV_STAGES[1:]) for side in (0, half)]
        pairs = [(wqkv_hbm.at[:, a:b], wqkv.at[:, a:b]) for a, b in spans]
        pairs += [(wo_hbm, wo), (w1_hbm, w1), (w2_hbm, w2), (b1_hbm, b1), (b2_hbm, b2)]
        w_copies = [pltpu.make_async_copy(src, dst, sem_w.at[n]) for n, (src, dst) in enumerate(pairs)]
        qkv_copies, other_copies = w_copies[:len(spans)], w_copies[len(spans):]

        def qkv_stage(n):
            qkv_copies[2 * n].wait()
            qkv_copies[2 * n + 1].wait()
            if n + 2 == len(QKV_STAGES):
                x_copy(1).wait()
                for i in range(2, NB):
                    x_copy(i).start()
            for job in qkv_mm.weight_jobs(wqkv, wqkv_op, range(QKV_STAGES[n], QKV_STAGES[n + 1])):
                job()

        def norm_jobs(src_ref, slot, mm, op_ref, step):
            def job(r):
                ys = []
                for i in range(mm.q):
                    a = i * mm.rows + r
                    ys.append(_ln(src_ref[a:a + step, :].astype(F32)))
                    xn.at[slot][_half(a, a + step), :] = _pack(ys[i])
                mm.put_input(lambda i, t: ys[i][:, _lanes(t)], op_ref.at[slot], r, r + step)
            return [functools.partial(job, r) for r in range(0, mm.rows, step)]

        def project(i, jobs, step):
            filler = _Filler()
            for part in jobs:
                if i > 0:
                    filler.add(part, 0, qkv_mm.work * 0.98)
                else:
                    filler.add(part, qkv_mm.work * (QKV_STAGES[-2] + 0.1) / qkv_mm.nq, qkv_mm.work * 0.94)
            row = lax.broadcasted_iota(I32, (KD, RB), 0)
            row8 = lax.broadcasted_iota(I32, (8, RB), 0)
            nd = D // LANE
            tiles, todo = {}, [(part, h) for part in range(3) for h in range(H)]

            def window(part, start, size, axis):
                pieces = []
                for t in range(start // LANE, (min(start + size, D) - 1) // LANE + 1):
                    a, b = max(start - t * LANE, 0), min(start + size - t * LANE, LANE)
                    pieces.append(lax.slice_in_dim(tiles[part, t], a, b, axis=axis))
                if start + size > D:
                    pieces.append(jnp.zeros_like(lax.slice_in_dim(pieces[0], 0, start + size - D, axis=axis)))
                return pieces[0] if len(pieces) == 1 else jnp.concatenate(pieces, axis=axis)

            for n, res in enumerate(qkv_mm.columns(xn.at[i % 2], xn_op.at[i % 2], wqkv, wqkv_op, filler, step, i > 0)):
                if i == 0 and n + 1 in QKV_STAGES[1:-1]:
                    qkv_stage(QKV_STAGES.index(n + 1))
                for t, val in res.items():
                    if t // nd == 0:
                        tiles[0, t % nd] = (val * QSCALE).T
                    elif t // nd == 1:
                        tiles[1, t % nd] = _pack(val)
                        if i == NB - 1:
                            tiles[3, t % nd] = val[RB - KPAD:].T
                    else:
                        tiles[2, t % nd] = val.T
                for part, h in list(todo):
                    b0 = 8 * (DH * h // 8)
                    if (part, b0 // LANE) not in tiles or (part, (min(b0 + KD, D) - 1) // LANE) not in tiles:
                        continue
                    todo.remove((part, h))
                    if part == 0:
                        lo = DH * h - b0
                        qw.at[h, i][...] = _pack(jnp.where((row >= lo) & (row < lo + DH), window(0, b0, KD, 0), 0.0))
                    elif part == 1:
                        kw[h, _half(i * RB, (i + 1) * RB), :] = window(1, b0, KD, 1)
                        if i == NB - 1:
                            kt[h] = window(3, b0, VR, 0)
                    elif h % 2 == 0:
                        vw[h, i, 0:16] = window(2, b0, 16, 0)
                        vw[h, i, 16:24] = jnp.where(row8 < 4, window(2, b0 + 16, 8, 0), 1.0)
                    else:
                        vw[h, i, 0:8] = jnp.where(row8 < 4, 1.0, window(2, b0, 8, 0))
                        vw[h, i, 8:24] = window(2, b0 + 8, 16, 0)
            assert not todo
            filler.flush()

        def first_blocks(n, carry):
            @pl.when(n == 0)
            def _():
                project(0, [norm_jobs(xv.at[1], 1, qkv_mm, xn_op, 32)], 256)

            @pl.when(n < 1)
            def _():
                for i in range(2, NB):
                    x_copy(i).wait()
                for c in other_copies:
                    c.start()

            @pl.when(n != 1)
            def _():
                for i in range(1, NB - 1):
                    project(i, [norm_jobs(xv.at[i + 1], (i + 1) % 2, qkv_mm, xn_op, 16)], 128)

            @pl.when(n + 1 == 1)
            def _():
                for c in other_copies:
                    c.wait()
            return carry

        x_copy(0).start()
        for c in qkv_copies[:2]:
            c.start()
        x_copy(0).wait()
        for c in qkv_copies[2:]:
            c.start()
        x_copy(1).start()
        for job in norm_jobs(xv.at[0], 0, qkv_mm, xn_op, 64):
            job()
        qkv_stage(0)
        lax.fori_loop(0, 2, first_blocks, 0)
        project(NB - 1, [out_mm.weight_jobs(wo, wo_op), down_mm.weight_jobs(w2, w2_op),
                         up_mm.weight_jobs(w1, w1_op)], 128)

        def attention(new, old, nxt, par, group):
            acc, pend, vacc = {}, {}, {}
            shared = old is not None
            bounds = [16 * ((mxu_keys if shared else S) // 16 * c // NT) for c in range(NT + 1)]

            def put(a, b, u, s):
                probs[par][_half(a, b), _lanes(u)] = _pack(jnp.exp2(s))

            def mxu_scores(c, u):
                k_ref, q_ref = new
                a, b = bounds[c], bounds[c + 1]
                put(a, b, u, _dot(_unpack(k_ref[_half(a, b), :]), _unpack(q_ref[u // TPB, :, _lanes(u % TPB)])))

            def vpu_scores(a0, u, d0, d1):
                sums = vacc.setdefault((a0, u), [None, None])
                for d in range(d0, d1):
                    q = qb[par][d, :, _lanes(u)]
                    for a in range(2):
                        t = kb[par][d, a0 + 8 * a:a0 + 8 * a + 8, :] * q
                        sums[a] = t if sums[a] is None else sums[a] + t
                if d1 == DH:
                    put(mxu_keys + a0, mxu_keys + a0 + 16, u, jnp.concatenate(sums, axis=0))

            def fetch(c, u):
                pend[c, u] = _unpack(probs[1 - par][_half(c * LANE, (c + 1) * LANE), _lanes(u)])

            def weigh(c, u):
                v_ref, o_ref = old
                o = _dot(v_ref[c // TPB, :, _lanes(c % TPB)], pend.pop((c, u)))
                acc[u] = acc[u] + o if c else o
                if c == NT - 1:
                    o_ref[u // TPB, :, _lanes(u % TPB)] = acc[u]

            def spread_k(d):
                r = d + 4 * (1 - par)
                kb[1 - par][d] = jnp.broadcast_to(nxt[0][r:r + 1, :], (LANE, KPAD)).T[KPAD - VPU_KEYS:]

            def spread_q(u):
                q = _unpack(nxt[1][u // TPB, :, _lanes(u % TPB)]).astype(F32)
                for d in range(DH):
                    r = d + 4 * (1 - par)
                    qb[1 - par][d, :, _lanes(u)] = jnp.broadcast_to(q[r:r + 1, :], (8, LANE))

            events = []
            for j in range(NT // group):
                t0 = j * NT * group
                cells = [(t0 + c * group + w, c, j * group + w) for c in range(NT) for w in range(group)]
                for t, c, u in cells if old is not None else []:
                    events.append((t - 4, 0, functools.partial(fetch, c, u)))
                    events.append((t, 1, functools.partial(weigh, c, u)))
                for t, c, u in cells if new is not None else []:
                    events.append((t - 3.5, 3, functools.partial(mxu_scores, c, u)))
                parts = [(a0, j * group + w, d, d + 2)
                         for a0 in range(0, VPU_KEYS, 16) for w in range(group) for d in range(0, DH, 2)]
                for n, part in enumerate(parts if new is not None and shared else []):
                    t = (t0 + NT * group * (n + 0.5) / len(parts)) * 99.0 / 100 + 3.0
                    events.append((t, 2, functools.partial(vpu_scores, *part)))
            if nxt is not None:
                for job, count, a, b in ((spread_k, DH, 20, 80), (spread_q, NT, 30, 80)):
                    for n in range(count):
                        events.append((NT * NT * (a + (b - a) * (n + 0.5) / count) / 100, 8, functools.partial(job, n)))
            events.sort(key=lambda e: e[:2])
            return [e[2] for e in events]

        def two_heads(j, carry):
            for par in (1, 0):
                h = 2 * j + 2 - par
                new, old, nxt = jnp.minimum(h, H - 1), h - 1, jnp.minimum(h + 1, H - 1)
                refs = (kw.at[new], qw.at[new]), (vw.at[old], oraw.at[old]), (kt.at[nxt], qw.at[nxt])

                @pl.when(h < H)
                def _():
                    for job in attention(*refs, par, NT):
                        job()
            return carry

        seen[0:2] = jnp.ones((2, 8, LANE), F32)
        seen[2] = jnp.zeros((8, LANE), F32)
        for job in attention((kw.at[0], qw.at[0]), None, (kt.at[1], qw.at[1]), 0, NT):
            job()
        lax.fori_loop(0, H // 2, two_heads, 0)

        def heads(i, u, h0, h1):
            row8 = lax.broadcasted_iota(I32, (8, LANE), 0)
            parts, sums = [], []
            for h in range(h0, h1, 2):
                e, o = oraw[h, i, :, _lanes(u)], oraw[h + 1, i, :, _lanes(u)]
                total = jnp.where(row8 < 4, o[0:8], e[16:24])
                inv = pl.reciprocal(total, approx=True)
                inv = inv * (2.0 - total * inv)
                parts += [e[0:16] * inv[4:5], jnp.where(row8 < 4, e[16:24], o[0:8]) * pltpu.roll(inv, 4, 0),
                          o[8:24] * inv[0:1]]
                sums.append(total)
            return jnp.concatenate(parts, axis=0), sums

        def gather_jobs(i, tiles):
            res, stats, n = {}, [], out_mm.rows // LANE

            def tile(u):
                h0 = tiles[0] * LANE // (2 * DH) * 2
                a, sums = heads(i, u, h0, min(H, (tiles[-1] + 1) * LANE // DH + 1))
                stats.append((functools.reduce(jnp.minimum, sums), functools.reduce(jnp.maximum, sums),
                              jnp.sum(a.reshape(-1, 8, LANE), axis=0)))
                for t in tiles:
                    res[u, t] = a[t * LANE - h0 * DH:(t + 1) * LANE - h0 * DH].T
                    att.at[i][_half(u * LANE, (u + 1) * LANE), _lanes(t)] = _pack(res[u, t])

            def operands(u, r):
                out_mm.put_input(lambda p, t: res[p * n + u, t][r:r + 32], att_op.at[i], u * LANE + r, u * LANE + r + 32)

            def record():
                lo, hi, total = zip(*stats)
                seen[0] = functools.reduce(jnp.minimum, lo, seen[0])
                seen[1] = functools.reduce(jnp.maximum, hi, seen[1])
                seen[2] = functools.reduce(jnp.add, total, seen[2])

            jobs = []
            for u in range(n):
                jobs += [functools.partial(tile, p * n + u) for p in range(out_mm.q)]
                if tiles[0] == 0:
                    jobs += [functools.partial(operands, u, r) for r in range(0, LANE, 32)]
            return jobs + [record]

        def mix(blocks, jobs, pending):
            spread = _Filler()
            spread.add(jobs, 0, out_mm.work * len(blocks) * 0.9)
            for i in blocks:
                filler = _Filler(spread)
                filler.add(gather_jobs(i, (4,)), 0, out_mm.rows * out_mm.kq * 5)
                if i == 0:
                    filler.add(pending, 0, out_mm.work * 0.95)
                if i + 1 < NB:
                    filler.add(gather_jobs(i + 1, (0, 1, 2, 3)), 0, out_mm.work * 0.85)
                for res in out_mm.columns(att.at[i], att_op.at[i], wo, wo_op, filler, 256):
                    for t, val in res.items():
                        hres[i, :, _lanes(t)] = xv[i, :, _lanes(t)].astype(F32) + val
                filler.flush()
            spread.flush()

        def project_heads(n, carry):
            @pl.when(n == 0)
            def _():
                last = attention(None, (vw.at[H - 1], oraw.at[H - 1]), None, H % 2, TPB)
                count = len(last) // NB + 8
                filler = _Filler()
                filler.add(gather_jobs(0, (0, 1, 2, 3)), 0, count)
                for job in last[:count]:
                    job()
                    filler.tick(1)
                filler.flush()
                mix(range(0, NB // 2), [], last[count:])

            @pl.when(n == 1)
            def _():
                mix(range(NB // 2, NB), norm_jobs(hres.at[0], 0, up_mm, hn_op, 16), [])
            return carry

        def feed_forward(i, carry):
            h_ref, next_ref, out_ref = hres.at[i], hres.at[jnp.minimum(i + 1, NB - 1)], xv.at[i]

            @pl.when(i != NB)
            def _():
                bias = b1[...].astype(F32).reshape(1, F)
                cols = {}
                for res in up_mm.columns(xn.at[0], hn_op.at[0], w1, w1_op, _Filler(), RB):
                    for t, val in res.items():
                        r = jnp.maximum(val + bias[:, _lanes(t)], 0.0)
                        cols[t] = r * r
                        act[:, _lanes(t)] = _pack(cols[t])
                    ready = [k for k in range(down_mm.kq) if k in cols and down_mm.kq + k in cols]
                    down_mm.put_input(lambda p, t: cols[t][p * down_mm.rows:(p + 1) * down_mm.rows],
                                      act_op.at[0], 0, down_mm.rows, ready)
                    for k in ready:
                        cols.pop(k)
                bias = b2[...].astype(F32).reshape(1, D)
                filler = _Filler()
                filler.add(norm_jobs(next_ref, 0, up_mm, hn_op, 16), 0, down_mm.work * 0.9)
                for res in down_mm.columns(act, act_op.at[0], w2, w2_op, filler, RB // 2):
                    for t, val in res.items():
                        out_ref[:, _lanes(t)] = (h_ref[:, _lanes(t)] + (val + bias[:, _lanes(t)])).astype(BF16)
                        o_copy(i, t).start()
                filler.flush()
            return carry

        lax.fori_loop(0, 2, project_heads, 0)
        lax.fori_loop(0, NB, feed_forward, 0)
        safe = (seen[0] >= SUM_MIN) & (seen[1] <= SUM_MAX) & (jnp.abs(seen[2]) <= 3e38)
        unsafe = jnp.max(jnp.where(safe, 0, 1)) > 0
        for i in range(NB):
            for t in range(D // LANE):
                o_copy(i, t).wait()

        @pl.when(unsafe)
        def _():
            def head(n, carry):
                h, i = n // NB, n % NB
                q = _unpack(qw[h, i])

                def scores(c):
                    rows = pl.ds(pl.multiple_of(c * (LANE // 2), LANE // 2), LANE // 2)
                    return _dot(_unpack(kw[h, rows, :]), q)

                m = lax.fori_loop(0, NT, lambda c, m: jnp.maximum(m, jnp.max(scores(c), axis=0, keepdims=True)),
                                  jnp.full((1, RB), -jnp.inf, F32))

                def weigh(b, o):
                    for c in range(TPB):
                        o = o + _dot(vw[h, b, :, _lanes(c)], jnp.exp2(scores(b * TPB + c) - m))
                    return o
                oraw[h, i] = lax.fori_loop(0, NB, weigh, jnp.zeros((VR, RB), F32))
                return carry
            lax.fori_loop(0, H * NB, head, 0)

            def block(i, carry):
                x_copy(i).start()
                x_copy(i).wait()
                for u in range(TPB):
                    att.at[0][_half(u * LANE, (u + 1) * LANE), :] = _pack(heads(i, u, 0, H)[0].T)

                def rows(r, carry):
                    at = pl.ds(pl.multiple_of(r * 32, 32), 32)
                    a = _unpack(att[0, pl.ds(pl.multiple_of(r * 16, 16), 16), :])
                    hh = xv[i, at, :].astype(F32) + _dot(a, wo[...])
                    g = jnp.maximum(_dot(_ln(hh).astype(BF16), w1[...]) + b1[...].astype(F32).reshape(1, F), 0.0)
                    out = hh + (_dot((g * g).astype(BF16), w2[...]) + b2[...].astype(F32).reshape(1, D))
                    xv[i, at, :] = out.astype(BF16)
                    return carry
                lax.fori_loop(0, RB // 32, rows, 0)
                done = pltpu.make_async_copy(xv.at[i], o_hbm.at[pl.ds(i * RB, RB)], sem_x.at[i])
                done.start()
                done.wait()
                return carry
            lax.fori_loop(0, NB, block, 0)

    scratch = [
        pltpu.VMEM((NB, RB, D), BF16),
        pltpu.VMEM((D, 3 * D), BF16), pltpu.VMEM((D, D), BF16), pltpu.VMEM((D, F), BF16), pltpu.VMEM((F, D), BF16),
        qkv_mm.weight_scratch(), out_mm.weight_scratch(), up_mm.weight_scratch(), down_mm.weight_scratch(),
        pltpu.VMEM((2, RB // 2, D), I32), qkv_mm.input_scratch(2), up_mm.input_scratch(1),
        pltpu.VMEM((NB, RB // 2, D), I32), out_mm.input_scratch(NB),
        pltpu.VMEM((RB // 2, F), I32), down_mm.input_scratch(1),
        pltpu.VMEM((NB, RB, D), F32),
        pltpu.VMEM((H, S // 2, KD), I32), pltpu.VMEM((H, VR, KPAD), F32),
        pltpu.VMEM((H, NB, KD // 2, RB), I32),
        pltpu.VMEM((H, NB, VR, RB), F32), pltpu.VMEM((H, NB, VR, RB), F32),
        pltpu.VMEM((4, 8, LANE), F32),
        pltpu.VMEM((S // 2, S), I32), pltpu.VMEM((S // 2, S), I32),
        pltpu.VMEM((DH, VPU_KEYS, LANE), F32), pltpu.VMEM((DH, VPU_KEYS, LANE), F32),
        pltpu.VMEM((DH, 8, S), F32), pltpu.VMEM((DH, 8, S), F32),
        pltpu.VMEM((F,), BF16), pltpu.VMEM((D,), BF16),
        pltpu.SemaphoreType.DMA((NB,)), pltpu.SemaphoreType.DMA((2 * len(QKV_STAGES) + 3,)), pltpu.SemaphoreType.DMA((NB * D // LANE,)),
    ]
    out = pl.pallas_call(
        kernel,
        out_shape=jax.ShapeDtypeStruct((S, D), BF16),
        in_specs=[pl.BlockSpec(memory_space=pl.ANY)] * 7,
        out_specs=pl.BlockSpec(memory_space=pl.ANY),
        scratch_shapes=scratch,
        compiler_params=pltpu.CompilerParams(
            vmem_limit_bytes=120 * 2**20, flags={"XLA_TPU_EVENLY_DISTRIBUTE_CRITICAL_NODES": True}),
    )(A_x.reshape(S, D), A_wqkv, A_wo, B_w1, B_b1, B_w2, B_b2)
    return out.reshape(1, S, D)
```

```python
import functools

import jax
import jax.numpy as jnp
from jax import lax
import jax.experimental.pallas as pl
import jax.experimental.pallas.tpu as pltpu

F32, BF16, I32 = jnp.float32, jnp.bfloat16, jnp.int32

S, D, F, H = 2048, 640, 1536, 32
DH = D // H
LANE = 128
NT = S // LANE
RB = 512
NB = S // RB
TPB = RB // LANE
KD = 32
VR = 24
EPS = 1e-5
QSCALE = float(DH ** -0.5 * 1.4426950408889634)
SUM_MIN, SUM_MAX = 2.0 ** -40, 2.0 ** 100

VPU_KEYS = 272
KPAD = 384
QKV_STAGES = (0, 2, 4, 7)

_A_TERMS = (((1, 0), (1, 3)), ((1, 3),), ((1, 0), (1, 1)), ((1, 1), (-1, 3)), ((1, 2), (1, 3)), ((1, 0),), ((1, 2), (-1, 0)))
_B_TERMS = (((1, 0), (1, 3)), ((1, 2), (-1, 0)), ((1, 3),), ((1, 2), (1, 3)), ((1, 0),), ((1, 1), (-1, 3)), ((1, 0), (1, 1)))
_C_TERMS = (((1, 0), (1, 3)), ((1, 0), (1, 2)), ((-1, 0), (1, 1)), ((1, 0),), ((1, 2), (-1, 3)), ((1, 1), (1, 3)), ((1, 3),))


def _ln(x):
    mean = jnp.mean(x, axis=-1, keepdims=True)
    xc = x - mean
    var = jnp.mean(xc * xc, axis=-1, keepdims=True)
    return xc * lax.rsqrt(var + EPS)


def _dot(a, b):
    return jnp.dot(a, b, preferred_element_type=F32)


def _lanes(u):
    return slice(u * LANE, (u + 1) * LANE)


def _pack(v):
    return pltpu.bitcast(v.astype(BF16), I32)


def _unpack(v):
    return pltpu.bitcast(v, BF16)


def _half(a, b):
    return slice(a // 2, b // 2)


def _operands(blocks, terms, level):
    if level == 0:
        return [blocks[0][0]]
    n = len(blocks) // 2
    out = []
    for (_, first), *rest in terms:
        def combine(i, j):
            val = blocks[first // 2 * n + i][first % 2 * n + j]
            for sign, q in rest:
                other = blocks[q // 2 * n + i][q % 2 * n + j]
                val = val + other if sign > 0 else val - other
            return val
        out += _operands([[combine(i, j) for j in range(n)] for i in range(n)], terms, level - 1)
    return out


def _combine(product):
    out = {}
    for r, term in enumerate(_C_TERMS):
        grid = product(r)
        n = len(grid)
        for sign, q in term:
            for i in range(n):
                for j in range(n):
                    key = (q // 2 * n + i, q % 2 * n + j)
                    if key not in out:
                        assert sign > 0, "every quadrant has to start with a positive term"
                        out[key] = grid[i][j]
                    else:
                        out[key] = out[key] + grid[i][j] if sign > 0 else out[key] - grid[i][j]
    return [[out[i, j] for j in range(2 * n)] for i in range(2 * n)]


class _Filler:
    def __init__(self, parent=None):
        self.jobs, self.now, self.parent = [], 0, parent

    def add(self, jobs, start, stop):
        self.jobs += [(start + (stop - start) * (n + 0.5) / len(jobs), job) for n, job in enumerate(jobs)]
        self.jobs.sort(key=lambda e: e[0])

    def tick(self, work):
        self.now += work
        if self.parent is not None:
            self.parent.tick(work)
        while self.jobs and self.jobs[0][0] <= self.now:
            self.jobs.pop(0)[1]()

    def flush(self):
        while self.jobs:
            self.jobs.pop(0)[1]()


class _Linear:
    def __init__(self, k, n, level):
        self.k, self.n, self.level, self.q = k, n, level, 2 ** level
        self.kq = k // (LANE * self.q)
        self.nq = n // (LANE * self.q)
        self.rows = RB // self.q
        self.work = (7 ** level * self.rows * self.kq * self.nq
                     + RB * ((k // LANE) * (n // LANE) - self.kq * self.nq * self.q ** 2))

    def weight_scratch(self):
        return pltpu.VMEM((7 ** self.level, self.kq * LANE // 2, self.nq * LANE), I32)

    def input_scratch(self, slots):
        return pltpu.VMEM((slots, 7 ** self.level, self.rows // 2, self.kq * LANE), I32)

    def weight_jobs(self, w_ref, op_ref, groups=None):
        part = self.kq * LANE

        def job(r0, j):
            blocks = [[w_ref[a * part + r0:a * part + r0 + 16, _lanes(b * self.nq + j)].astype(F32)
                       for b in range(self.q)] for a in range(self.q)]
            for r, op in enumerate(_operands(blocks, _B_TERMS, self.level)):
                op_ref.at[r][_half(r0, r0 + 16), _lanes(j)] = _pack(op)
        return [functools.partial(job, r0, j) for j in (range(self.nq) if groups is None else groups)
                for r0 in range(0, part, 16)]

    def put_input(self, block, op_ref, r0, r1, tiles=None):
        for kt in range(self.kq) if tiles is None else tiles:
            blocks = [[block(i, b * self.kq + kt) for b in range(self.q)] for i in range(self.q)]
            for r, op in enumerate(_operands(blocks, _A_TERMS, self.level)):
                op_ref.at[r][_half(r0, r1), _lanes(kt)] = _pack(op)

    def columns(self, a_ref, aop_ref, w_ref, wop_ref, filler, step, rest_first=False):
        def dot(a, b):
            out = _dot(a, b)
            filler.tick(a.shape[0] * a.shape[1] // LANE)
            return out

        def direct(t, k0):
            return jnp.concatenate([dot(_unpack(a_ref[_half(m, m + step), k0:self.k]), w_ref[k0:self.k, _lanes(t)])
                                    for m in range(0, RB, step)], axis=0)

        k0 = self.kq * self.q * LANE
        for j in range(self.nq):
            tiles = [b * self.nq + j for b in range(self.q)]
            rest = {t: direct(t, k0) for t in tiles if rest_first}

            def product(r):
                return [[dot(_unpack(aop_ref[r]), _unpack(wop_ref[r, :, _lanes(j)]))]]
            if self.level == 1:
                grid = _combine(product)
            else:
                grid = _combine(lambda r: _combine(lambda s: product(7 * r + s)))
            out = {}
            for b, t in enumerate(tiles):
                out[t] = jnp.concatenate([row[b] for row in grid], axis=0)
                if k0 < self.k:
                    out[t] = out[t] + (rest[t] if rest_first else direct(t, k0))
            yield out
        for t in range(self.nq * self.q, self.n // LANE):
            yield {t: direct(t, 0)}


@jax.jit
def pallas_sequential_preLN__softmax_full_mha__dense_activation_squared_relu__prompt_kernel(
    A_x: jax.Array,
    A_wqkv: jax.Array,
    A_wo: jax.Array,
    B_x: jax.Array,
    B_w1: jax.Array,
    B_b1: jax.Array,
    B_w2: jax.Array,
    B_b2: jax.Array,
):
    del B_x
    mxu_keys = S - VPU_KEYS
    qkv_mm, out_mm = _Linear(D, 3 * D, 1), _Linear(D, D, 1)
    up_mm, down_mm = _Linear(D, F, 2), _Linear(F, D, 1)

    def kernel(x_hbm, wqkv_hbm, wo_hbm, w1_hbm, b1_hbm, w2_hbm, b2_hbm, o_hbm,
               xv, wqkv, wo, w1, w2, wqkv_op, wo_op, w1_op, w2_op, xn, xn_op, hn_op, att, att_op, act, act_op,
               hres, kw, kt, qw, vw, oraw, seen, p0, p1, kb0, kb1, qb0, qb1, b1, b2, sem_x, sem_w, sem_o):
        probs, kb, qb = (p0, p1), (kb0, kb1), (qb0, qb1)

        def x_copy(i):
            return pltpu.make_async_copy(x_hbm.at[pl.ds(i * RB, RB)], xv.at[i], sem_x.at[i])

        def o_copy(i, t):
            return pltpu.make_async_copy(xv.at[i, :, _lanes(t)], o_hbm.at[pl.ds(i * RB, RB), _lanes(t)],
                                         sem_o.at[i * (D // LANE) + t])

        half = qkv_mm.nq * LANE
        spans = [(side + a * LANE, side + b * LANE if b < qkv_mm.nq or not side else 3 * D)
                 for a, b in zip(QKV_STAGES, QKV_STAGES[1:]) for side in (0, half)]
        pairs = [(wqkv_hbm.at[:, a:b], wqkv.at[:, a:b]) for a, b in spans]
        pairs += [(wo_hbm, wo), (w1_hbm, w1), (w2_hbm, w2), (b1_hbm, b1), (b2_hbm, b2)]
        w_copies = [pltpu.make_async_copy(src, dst, sem_w.at[n]) for n, (src, dst) in enumerate(pairs)]
        qkv_copies, other_copies = w_copies[:len(spans)], w_copies[len(spans):]

        def qkv_stage(n):
            qkv_copies[2 * n].wait()
            qkv_copies[2 * n + 1].wait()
            if n + 2 == len(QKV_STAGES):
                x_copy(1).wait()
                for i in range(2, NB):
                    x_copy(i).start()
            for job in qkv_mm.weight_jobs(wqkv, wqkv_op, range(QKV_STAGES[n], QKV_STAGES[n + 1])):
                job()

        def norm_jobs(src_ref, slot, mm, op_ref, step):
            def job(r):
                ys = []
                for i in range(mm.q):
                    a = i * mm.rows + r
                    ys.append(_ln(src_ref[a:a + step, :].astype(F32)))
                    xn.at[slot][_half(a, a + step), :] = _pack(ys[i])
                mm.put_input(lambda i, t: ys[i][:, _lanes(t)], op_ref.at[slot], r, r + step)
            return [functools.partial(job, r) for r in range(0, mm.rows, step)]

        def project(i, jobs, step):
            filler = _Filler()
            for part in jobs:
                if i > 0:
                    filler.add(part, 0, qkv_mm.work * 0.98)
                else:
                    filler.add(part, qkv_mm.work * (QKV_STAGES[-2] + 0.1) / qkv_mm.nq, qkv_mm.work * 0.94)
            row = lax.broadcasted_iota(I32, (KD, RB), 0)
            row8 = lax.broadcasted_iota(I32, (8, RB), 0)
            nd = D // LANE
            tiles, todo = {}, [(part, h) for part in range(3) for h in range(H)]

            def window(part, start, size, axis):
                pieces = []
                for t in range(start // LANE, (min(start + size, D) - 1) // LANE + 1):
                    a, b = max(start - t * LANE, 0), min(start + size - t * LANE, LANE)
                    pieces.append(lax.slice_in_dim(tiles[part, t], a, b, axis=axis))
                if start + size > D:
                    pieces.append(jnp.zeros_like(lax.slice_in_dim(pieces[0], 0, start + size - D, axis=axis)))
                return pieces[0] if len(pieces) == 1 else jnp.concatenate(pieces, axis=axis)

            for n, res in enumerate(qkv_mm.columns(xn.at[i % 2], xn_op.at[i % 2], wqkv, wqkv_op, filler, step, i > 0)):
                if i == 0 and n + 1 in QKV_STAGES[1:-1]:
                    qkv_stage(QKV_STAGES.index(n + 1))
                for t, val in res.items():
                    if t // nd == 0:
                        tiles[0, t % nd] = (val * QSCALE).T
                    elif t // nd == 1:
                        tiles[1, t % nd] = _pack(val)
                        if i == NB - 1:
                            tiles[3, t % nd] = val[RB - KPAD:].T
                    else:
                        tiles[2, t % nd] = val.T
                for part, h in list(todo):
                    b0 = 8 * (DH * h // 8)
                    if (part, b0 // LANE) not in tiles or (part, (min(b0 + KD, D) - 1) // LANE) not in tiles:
                        continue
                    todo.remove((part, h))
                    if part == 0:
                        lo = DH * h - b0
                        qw.at[h, i][...] = _pack(jnp.where((row >= lo) & (row < lo + DH), window(0, b0, KD, 0), 0.0))
                    elif part == 1:
                        kw[h, _half(i * RB, (i + 1) * RB), :] = window(1, b0, KD, 1)
                        if i == NB - 1:
                            kt[h] = window(3, b0, VR, 0)
                    elif h % 2 == 0:
                        vw[h, i, 0:16] = window(2, b0, 16, 0)
                        vw[h, i, 16:24] = jnp.where(row8 < 4, window(2, b0 + 16, 8, 0), 1.0)
                    else:
                        vw[h, i, 0:8] = jnp.where(row8 < 4, 1.0, window(2, b0, 8, 0))
                        vw[h, i, 8:24] = window(2, b0 + 8, 16, 0)
            assert not todo
            filler.flush()

        def first_blocks(n, carry):
            @pl.when(n == 0)
            def _():
                project(0, [norm_jobs(xv.at[1], 1, qkv_mm, xn_op, 32)], 256)

            @pl.when(n < 1)
            def _():
                for i in range(2, NB):
                    x_copy(i).wait()
                for c in other_copies:
                    c.start()

            @pl.when(n != 1)
            def _():
                for i in range(1, NB - 1):
                    project(i, [norm_jobs(xv.at[i + 1], (i + 1) % 2, qkv_mm, xn_op, 16)], 128)

            @pl.when(n + 1 == 1)
            def _():
                for c in other_copies:
                    c.wait()
            return carry

        x_copy(0).start()
        for c in qkv_copies[:2]:
            c.start()
        x_copy(0).wait()
        for c in qkv_copies[2:]:
            c.start()
        x_copy(1).start()
        for job in norm_jobs(xv.at[0], 0, qkv_mm, xn_op, 64):
            job()
        qkv_stage(0)
        lax.fori_loop(0, 2, first_blocks, 0)
        project(NB - 1, [out_mm.weight_jobs(wo, wo_op), down_mm.weight_jobs(w2, w2_op),
                         up_mm.weight_jobs(w1, w1_op)], 128)

        def attention(new, old, nxt, par, group):
            acc, pend, vacc = {}, {}, {}
            shared = old is not None
            bounds = [16 * ((mxu_keys if shared else S) // 16 * c // NT) for c in range(NT + 1)]

            def put(a, b, u, s):
                probs[par][_half(a, b), _lanes(u)] = _pack(jnp.exp2(s))

            def mxu_scores(c, u):
                k_ref, q_ref = new
                a, b = bounds[c], bounds[c + 1]
                put(a, b, u, _dot(_unpack(k_ref[_half(a, b), :]), _unpack(q_ref[u // TPB, :, _lanes(u % TPB)])))

            def vpu_scores(a0, u, d):
                sums = vacc.setdefault((a0, u), [None, None])
                q = qb[par][d, :, _lanes(u)]
                for a in range(2):
                    t = kb[par][d, a0 + 8 * a:a0 + 8 * a + 8, :] * q
                    sums[a] = sums[a] + t if d else t
                if d == DH - 1:
                    put(mxu_keys + a0, mxu_keys + a0 + 16, u, jnp.concatenate(sums, axis=0))

            def fetch(c, u):
                pend[c, u] = _unpack(probs[1 - par][_half(c * LANE, (c + 1) * LANE), _lanes(u)])

            def weigh(c, u):
                v_ref, o_ref = old
                o = _dot(v_ref[c // TPB, :, _lanes(c % TPB)], pend.pop((c, u)))
                acc[u] = acc[u] + o if c else o
                if c == NT - 1:
                    o_ref[u // TPB, :, _lanes(u % TPB)] = acc[u]

            def spread_k(d):
                r = d + 4 * (1 - par)
                kb[1 - par][d] = jnp.broadcast_to(nxt[0][r:r + 1, :], (LANE, KPAD)).T[KPAD - VPU_KEYS:]

            def spread_q(u):
                q = _unpack(nxt[1][u // TPB, :, _lanes(u % TPB)]).astype(F32)
                for d in range(DH):
                    r = d + 4 * (1 - par)
                    qb[1 - par][d, :, _lanes(u)] = jnp.broadcast_to(q[r:r + 1, :], (8, LANE))

            events = []
            for j in range(NT // group):
                t0 = j * NT * group
                cells = [(t0 + c * group + w, c, j * group + w) for c in range(NT) for w in range(group)]
                pairs = [(c + k, j * group + w) for c in range(0, NT, 2) for w in range(group) for k in range(2)]
                for t, (c, u) in enumerate(pairs if old is not None else [], t0):
                    events.append((t - 4, 0, functools.partial(fetch, c, u)))
                    events.append((t, 1, functools.partial(weigh, c, u)))
                for t, c, u in cells if new is not None else []:
                    events.append((t - 4, 3, functools.partial(mxu_scores, c, u)))
                parts = [(a0, j * group + w, d)
                         for a0 in range(0, VPU_KEYS, 16) for w in range(group) for d in range(DH)]
                for n, part in enumerate(parts if new is not None and shared else []):
                    t = (t0 + NT * group * (n + 0.5) / len(parts)) * 98.8 / 100 + 3.0
                    events.append((t, 2, functools.partial(vpu_scores, *part)))
            if nxt is not None:
                for job, count, a, b in ((spread_k, DH, 20, 50), (spread_q, NT, 30, 80)):
                    for n in range(count):
                        events.append((NT * NT * (a + (b - a) * (n + 0.5) / count) / 100, 8, functools.partial(job, n)))
            events.sort(key=lambda e: e[:2])
            return [e[2] for e in events]

        def two_heads(j, carry):
            for par in (1, 0):
                h = 2 * j + 2 - par
                new, old, nxt = jnp.minimum(h, H - 1), h - 1, jnp.minimum(h + 1, H - 1)
                refs = (kw.at[new], qw.at[new]), (vw.at[old], oraw.at[old]), (kt.at[nxt], qw.at[nxt])

                @pl.when(h < H)
                def _():
                    for job in attention(*refs, par, NT):
                        job()
            return carry

        seen[0:2] = jnp.ones((2, 8, LANE), F32)
        seen[2] = jnp.zeros((8, LANE), F32)
        for job in attention((kw.at[0], qw.at[0]), None, (kt.at[1], qw.at[1]), 0, NT):
            job()
        lax.fori_loop(0, H // 2, two_heads, 0)

        def heads(i, u, h0, h1):
            row8 = lax.broadcasted_iota(I32, (8, LANE), 0)
            parts, sums = [], []
            for h in range(h0, h1, 2):
                e, o = oraw[h, i, :, _lanes(u)], oraw[h + 1, i, :, _lanes(u)]
                total = jnp.where(row8 < 4, o[0:8], e[16:24])
                inv = pl.reciprocal(total, approx=True)
                inv = inv * (2.0 - total * inv)
                parts += [e[0:16] * inv[4:5], jnp.where(row8 < 4, e[16:24], o[0:8]) * pltpu.roll(inv, 4, 0),
                          o[8:24] * inv[0:1]]
                sums.append(total)
            return jnp.concatenate(parts, axis=0), sums

        def gather_jobs(i, tiles):
            res, stats, n = {}, [], out_mm.rows // LANE

            def tile(u):
                h0 = tiles[0] * LANE // (2 * DH) * 2
                a, sums = heads(i, u, h0, min(H, (tiles[-1] + 1) * LANE // DH + 1))
                stats.append((functools.reduce(jnp.minimum, sums), functools.reduce(jnp.maximum, sums),
                              jnp.sum(a.reshape(-1, 8, LANE), axis=0)))
                for t in tiles:
                    res[u, t] = a[t * LANE - h0 * DH:(t + 1) * LANE - h0 * DH].T
                    att.at[i][_half(u * LANE, (u + 1) * LANE), _lanes(t)] = _pack(res[u, t])

            def operands(u, r):
                out_mm.put_input(lambda p, t: res[p * n + u, t][r:r + 32], att_op.at[i], u * LANE + r, u * LANE + r + 32)

            def record():
                lo, hi, total = zip(*stats)
                seen[0] = functools.reduce(jnp.minimum, lo, seen[0])
                seen[1] = functools.reduce(jnp.maximum, hi, seen[1])
                seen[2] = functools.reduce(jnp.add, total, seen[2])

            jobs = []
            for u in range(n):
                jobs += [functools.partial(tile, p * n + u) for p in range(out_mm.q)]
                if tiles[0] == 0:
                    jobs += [functools.partial(operands, u, r) for r in range(0, LANE, 32)]
            return jobs + [record]

        def mix(blocks, jobs, pending):
            spread = _Filler()
            spread.add(jobs, 0, out_mm.work * len(blocks) * 0.9)
            for i in blocks:
                filler = _Filler(spread)
                filler.add(gather_jobs(i, (4,)), 0, out_mm.rows * out_mm.kq * 5)
                if i == 0:
                    filler.add(pending, 0, out_mm.work * 0.95)
                if i + 1 < NB:
                    filler.add(gather_jobs(i + 1, (0, 1, 2, 3)), 0, out_mm.work * 0.85)
                for res in out_mm.columns(att.at[i], att_op.at[i], wo, wo_op, filler, 256):
                    for t, val in res.items():
                        hres[i, :, _lanes(t)] = xv[i, :, _lanes(t)].astype(F32) + val
                filler.flush()
            spread.flush()

        def project_heads(n, carry):
            @pl.when(n == 0)
            def _():
                last = attention(None, (vw.at[H - 1], oraw.at[H - 1]), None, H % 2, TPB)
                count = len(last) // NB + 8
                filler = _Filler()
                filler.add(gather_jobs(0, (0, 1, 2, 3)), 0, count)
                for job in last[:count]:
                    job()
                    filler.tick(1)
                filler.flush()
                mix(range(0, NB // 2), [], last[count:])

            @pl.when(n == 1)
            def _():
                mix(range(NB // 2, NB), norm_jobs(hres.at[0], 0, up_mm, hn_op, 16), [])
            return carry

        def feed_forward(i, carry):
            h_ref, next_ref, out_ref = hres.at[i], hres.at[jnp.minimum(i + 1, NB - 1)], xv.at[i]

            @pl.when(i != NB)
            def _():
                bias = b1[...].astype(F32).reshape(1, F)
                cols = {}
                for res in up_mm.columns(xn.at[0], hn_op.at[0], w1, w1_op, _Filler(), RB):
                    for t, val in res.items():
                        r = jnp.maximum(val + bias[:, _lanes(t)], 0.0)
                        cols[t] = r * r
                        act[:, _lanes(t)] = _pack(cols[t])
                    ready = [k for k in range(down_mm.kq) if k in cols and down_mm.kq + k in cols]
                    down_mm.put_input(lambda p, t: cols[t][p * down_mm.rows:(p + 1) * down_mm.rows],
                                      act_op.at[0], 0, down_mm.rows, ready)
                    for k in ready:
                        cols.pop(k)
                bias = b2[...].astype(F32).reshape(1, D)
                filler = _Filler()
                filler.add(norm_jobs(next_ref, 0, up_mm, hn_op, 16), 0, down_mm.work * 0.9)
                for res in down_mm.columns(act, act_op.at[0], w2, w2_op, filler, RB // 2):
                    for t, val in res.items():
                        out_ref[:, _lanes(t)] = (h_ref[:, _lanes(t)] + (val + bias[:, _lanes(t)])).astype(BF16)
                        o_copy(i, t).start()
                filler.flush()
            return carry

        lax.fori_loop(0, 2, project_heads, 0)
        lax.fori_loop(0, NB, feed_forward, 0)
        safe = (seen[0] >= SUM_MIN) & (seen[1] <= SUM_MAX) & (jnp.abs(seen[2]) <= 3e38)
        unsafe = jnp.max(jnp.where(safe, 0, 1)) > 0
        for i in range(NB):
            for t in range(D // LANE):
                o_copy(i, t).wait()

        @pl.when(unsafe)
        def _():
            def head(n, carry):
                h, i = n // NB, n % NB
                q = _unpack(qw[h, i])

                def scores(c):
                    rows = pl.ds(pl.multiple_of(c * (LANE // 2), LANE // 2), LANE // 2)
                    return _dot(_unpack(kw[h, rows, :]), q)

                m = lax.fori_loop(0, NT, lambda c, m: jnp.maximum(m, jnp.max(scores(c), axis=0, keepdims=True)),
                                  jnp.full((1, RB), -jnp.inf, F32))

                def weigh(b, o):
                    for c in range(TPB):
                        o = o + _dot(vw[h, b, :, _lanes(c)], jnp.exp2(scores(b * TPB + c) - m))
                    return o
                oraw[h, i] = lax.fori_loop(0, NB, weigh, jnp.zeros((VR, RB), F32))
                return carry
            lax.fori_loop(0, H * NB, head, 0)

            def block(i, carry):
                x_copy(i).start()
                x_copy(i).wait()
                for u in range(TPB):
                    att.at[0][_half(u * LANE, (u + 1) * LANE), :] = _pack(heads(i, u, 0, H)[0].T)

                def rows(r, carry):
                    at = pl.ds(pl.multiple_of(r * 32, 32), 32)
                    a = _unpack(att[0, pl.ds(pl.multiple_of(r * 16, 16), 16), :])
                    hh = xv[i, at, :].astype(F32) + _dot(a, wo[...])
                    g = jnp.maximum(_dot(_ln(hh).astype(BF16), w1[...]) + b1[...].astype(F32).reshape(1, F), 0.0)
                    out = hh + (_dot((g * g).astype(BF16), w2[...]) + b2[...].astype(F32).reshape(1, D))
                    xv[i, at, :] = out.astype(BF16)
                    return carry
                lax.fori_loop(0, RB // 32, rows, 0)
                done = pltpu.make_async_copy(xv.at[i], o_hbm.at[pl.ds(i * RB, RB)], sem_x.at[i])
                done.start()
                done.wait()
                return carry
            lax.fori_loop(0, NB, block, 0)

    scratch = [
        pltpu.VMEM((NB, RB, D), BF16),
        pltpu.VMEM((D, 3 * D), BF16), pltpu.VMEM((D, D), BF16), pltpu.VMEM((D, F), BF16), pltpu.VMEM((F, D), BF16),
        qkv_mm.weight_scratch(), out_mm.weight_scratch(), up_mm.weight_scratch(), down_mm.weight_scratch(),
        pltpu.VMEM((2, RB // 2, D), I32), qkv_mm.input_scratch(2), up_mm.input_scratch(1),
        pltpu.VMEM((NB, RB // 2, D), I32), out_mm.input_scratch(NB),
        pltpu.VMEM((RB // 2, F), I32), down_mm.input_scratch(1),
        pltpu.VMEM((NB, RB, D), F32),
        pltpu.VMEM((H, S // 2, KD), I32), pltpu.VMEM((H, VR, KPAD), F32),
        pltpu.VMEM((H, NB, KD // 2, RB), I32),
        pltpu.VMEM((H, NB, VR, RB), F32), pltpu.VMEM((H, NB, VR, RB), F32),
        pltpu.VMEM((4, 8, LANE), F32),
        pltpu.VMEM((S // 2, S), I32), pltpu.VMEM((S // 2, S), I32),
        pltpu.VMEM((DH, VPU_KEYS, LANE), F32), pltpu.VMEM((DH, VPU_KEYS, LANE), F32),
        pltpu.VMEM((DH, 8, S), F32), pltpu.VMEM((DH, 8, S), F32),
        pltpu.VMEM((F,), BF16), pltpu.VMEM((D,), BF16),
        pltpu.SemaphoreType.DMA((NB,)), pltpu.SemaphoreType.DMA((2 * len(QKV_STAGES) + 3,)), pltpu.SemaphoreType.DMA((NB * D // LANE,)),
    ]
    out = pl.pallas_call(
        kernel,
        out_shape=jax.ShapeDtypeStruct((S, D), BF16),
        in_specs=[pl.BlockSpec(memory_space=pl.ANY)] * 7,
        out_specs=pl.BlockSpec(memory_space=pl.ANY),
        scratch_shapes=scratch,
        compiler_params=pltpu.CompilerParams(
            vmem_limit_bytes=120 * 2**20, flags={"XLA_TPU_EVENLY_DISTRIBUTE_CRITICAL_NODES": True}),
    )(A_x.reshape(S, D), A_wqkv, A_wo, B_w1, B_b1, B_w2, B_b2)
    return out.reshape(1, S, D)
```

```python
import functools

import jax
import jax.numpy as jnp
from jax import lax
import jax.experimental.pallas as pl
import jax.experimental.pallas.tpu as pltpu

F32, BF16, I32 = jnp.float32, jnp.bfloat16, jnp.int32

S, D, F, H = 2048, 640, 1536, 32
DH = D // H
LANE = 128
NT = S // LANE
RB = 512
NB = S // RB
TPB = RB // LANE
KD = 32
VR = 24
EPS = 1e-5
QSCALE = float(DH ** -0.5 * 1.4426950408889634)
SUM_MIN, SUM_MAX = 2.0 ** -40, 2.0 ** 100

VPU_KEYS = 288
KPAD = 384
QKV_STAGES = (0, 2, 4, 7)

_A_TERMS = (((1, 0), (1, 3)), ((1, 3),), ((1, 0), (1, 1)), ((1, 1), (-1, 3)), ((1, 2), (1, 3)), ((1, 0),), ((1, 2), (-1, 0)))
_B_TERMS = (((1, 0), (1, 3)), ((1, 2), (-1, 0)), ((1, 3),), ((1, 2), (1, 3)), ((1, 0),), ((1, 1), (-1, 3)), ((1, 0), (1, 1)))
_C_TERMS = (((1, 0), (1, 3)), ((1, 0), (1, 2)), ((-1, 0), (1, 1)), ((1, 0),), ((1, 2), (-1, 3)), ((1, 1), (1, 3)), ((1, 3),))


def _ln(x):
    mean = jnp.mean(x, axis=-1, keepdims=True)
    xc = x - mean
    var = jnp.mean(xc * xc, axis=-1, keepdims=True)
    return xc * lax.rsqrt(var + EPS)


def _dot(a, b):
    return jnp.dot(a, b, preferred_element_type=F32)


def _lanes(u):
    return slice(u * LANE, (u + 1) * LANE)


def _pack(v):
    return pltpu.bitcast(v.astype(BF16), I32)


def _unpack(v):
    return pltpu.bitcast(v, BF16)


def _half(a, b):
    return slice(a // 2, b // 2)


def _operands(blocks, terms, level):
    if level == 0:
        return [blocks[0][0]]
    n = len(blocks) // 2
    out = []
    for (_, first), *rest in terms:
        def combine(i, j):
            val = blocks[first // 2 * n + i][first % 2 * n + j]
            for sign, q in rest:
                other = blocks[q // 2 * n + i][q % 2 * n + j]
                val = val + other if sign > 0 else val - other
            return val
        out += _operands([[combine(i, j) for j in range(n)] for i in range(n)], terms, level - 1)
    return out


def _combine(product):
    out = {}
    for r, term in enumerate(_C_TERMS):
        grid = product(r)
        n = len(grid)
        for sign, q in term:
            for i in range(n):
                for j in range(n):
                    key = (q // 2 * n + i, q % 2 * n + j)
                    if key not in out:
                        assert sign > 0, "every quadrant has to start with a positive term"
                        out[key] = grid[i][j]
                    else:
                        out[key] = out[key] + grid[i][j] if sign > 0 else out[key] - grid[i][j]
    return [[out[i, j] for j in range(2 * n)] for i in range(2 * n)]


class _Filler:
    def __init__(self, parent=None):
        self.jobs, self.now, self.parent = [], 0, parent

    def add(self, jobs, start, stop):
        self.jobs += [(start + (stop - start) * (n + 0.5) / len(jobs), job) for n, job in enumerate(jobs)]
        self.jobs.sort(key=lambda e: e[0])

    def tick(self, work):
        self.now += work
        if self.parent is not None:
            self.parent.tick(work)
        while self.jobs and self.jobs[0][0] <= self.now:
            self.jobs.pop(0)[1]()

    def flush(self):
        while self.jobs:
            self.jobs.pop(0)[1]()


class _Linear:
    def __init__(self, k, n, level):
        self.k, self.n, self.level, self.q = k, n, level, 2 ** level
        self.kq = k // (LANE * self.q)
        self.nq = n // (LANE * self.q)
        self.rows = RB // self.q
        self.work = (7 ** level * self.rows * self.kq * self.nq
                     + RB * ((k // LANE) * (n // LANE) - self.kq * self.nq * self.q ** 2))

    def weight_scratch(self):
        return pltpu.VMEM((7 ** self.level, self.kq * LANE // 2, self.nq * LANE), I32)

    def input_scratch(self, slots):
        return pltpu.VMEM((slots, 7 ** self.level, self.rows // 2, self.kq * LANE), I32)

    def weight_jobs(self, w_ref, op_ref, groups=None):
        part = self.kq * LANE

        def job(r0, j):
            blocks = [[w_ref[a * part + r0:a * part + r0 + 16, _lanes(b * self.nq + j)].astype(F32)
                       for b in range(self.q)] for a in range(self.q)]
            for r, op in enumerate(_operands(blocks, _B_TERMS, self.level)):
                op_ref.at[r][_half(r0, r0 + 16), _lanes(j)] = _pack(op)
        return [functools.partial(job, r0, j) for j in (range(self.nq) if groups is None else groups)
                for r0 in range(0, part, 16)]

    def put_input(self, block, op_ref, r0, r1, tiles=None):
        for kt in range(self.kq) if tiles is None else tiles:
            blocks = [[block(i, b * self.kq + kt) for b in range(self.q)] for i in range(self.q)]
            for r, op in enumerate(_operands(blocks, _A_TERMS, self.level)):
                op_ref.at[r][_half(r0, r1), _lanes(kt)] = _pack(op)

    def columns(self, a_ref, aop_ref, w_ref, wop_ref, filler, step, rest_first=False):
        def dot(a, b):
            out = _dot(a, b)
            filler.tick(a.shape[0] * a.shape[1] // LANE)
            return out

        def direct(t, k0):
            return jnp.concatenate([dot(_unpack(a_ref[_half(m, m + step), k0:self.k]), w_ref[k0:self.k, _lanes(t)])
                                    for m in range(0, RB, step)], axis=0)

        k0 = self.kq * self.q * LANE
        for j in range(self.nq):
            tiles = [b * self.nq + j for b in range(self.q)]
            rest = {t: direct(t, k0) for t in tiles if rest_first}

            def product(r):
                return [[dot(_unpack(aop_ref[r]), _unpack(wop_ref[r, :, _lanes(j)]))]]
            if self.level == 1:
                grid = _combine(product)
            else:
                grid = _combine(lambda r: _combine(lambda s: product(7 * r + s)))
            out = {}
            for b, t in enumerate(tiles):
                out[t] = jnp.concatenate([row[b] for row in grid], axis=0)
                if k0 < self.k:
                    out[t] = out[t] + (rest[t] if rest_first else direct(t, k0))
            yield out
        for t in range(self.nq * self.q, self.n // LANE):
            yield {t: direct(t, 0)}


@jax.jit
def pallas_sequential_preLN__softmax_full_mha__dense_activation_squared_relu__prompt_kernel(
    A_x: jax.Array,
    A_wqkv: jax.Array,
    A_wo: jax.Array,
    B_x: jax.Array,
    B_w1: jax.Array,
    B_b1: jax.Array,
    B_w2: jax.Array,
    B_b2: jax.Array,
):
    del B_x
    mxu_keys = S - VPU_KEYS
    qkv_mm, out_mm = _Linear(D, 3 * D, 1), _Linear(D, D, 1)
    up_mm, down_mm = _Linear(D, F, 2), _Linear(F, D, 1)

    def kernel(x_hbm, wqkv_hbm, wo_hbm, w1_hbm, b1_hbm, w2_hbm, b2_hbm, o_hbm,
               xv, wqkv, wo, w1, w2, wqkv_op, wo_op, w1_op, w2_op, xn, xn_op, hn_op, att, att_op, act, act_op,
               hres, kw, kt, qw, vw, oraw, seen, p0, p1, kb0, kb1, qb0, qb1, b1, b2, sem_x, sem_w, sem_o):
        probs, kb, qb = (p0, p1), (kb0, kb1), (qb0, qb1)

        def x_copy(i):
            return pltpu.make_async_copy(x_hbm.at[pl.ds(i * RB, RB)], xv.at[i], sem_x.at[i])

        def o_copy(i, t):
            return pltpu.make_async_copy(xv.at[i, :, _lanes(t)], o_hbm.at[pl.ds(i * RB, RB), _lanes(t)],
                                         sem_o.at[i * (D // LANE) + t])

        half = qkv_mm.nq * LANE
        spans = [(side + a * LANE, side + b * LANE if b < qkv_mm.nq or not side else 3 * D)
                 for a, b in zip(QKV_STAGES, QKV_STAGES[1:]) for side in (0, half)]
        pairs = [(wqkv_hbm.at[:, a:b], wqkv.at[:, a:b]) for a, b in spans]
        pairs += [(wo_hbm, wo), (w1_hbm, w1), (w2_hbm, w2), (b1_hbm, b1), (b2_hbm, b2)]
        w_copies = [pltpu.make_async_copy(src, dst, sem_w.at[n]) for n, (src, dst) in enumerate(pairs)]
        qkv_copies, other_copies = w_copies[:len(spans)], w_copies[len(spans):]

        def qkv_stage(n):
            qkv_copies[2 * n].wait()
            qkv_copies[2 * n + 1].wait()
            if n + 2 == len(QKV_STAGES):
                x_copy(1).wait()
                for i in range(2, NB):
                    x_copy(i).start()
            for job in qkv_mm.weight_jobs(wqkv, wqkv_op, range(QKV_STAGES[n], QKV_STAGES[n + 1])):
                job()

        def norm_jobs(src_ref, slot, mm, op_ref, step):
            def job(r):
                ys = []
                for i in range(mm.q):
                    a = i * mm.rows + r
                    ys.append(_ln(src_ref[a:a + step, :].astype(F32)))
                    xn.at[slot][_half(a, a + step), :] = _pack(ys[i])
                mm.put_input(lambda i, t: ys[i][:, _lanes(t)], op_ref.at[slot], r, r + step)
            return [functools.partial(job, r) for r in range(0, mm.rows, step)]

        def project(i, jobs, step):
            filler = _Filler()
            for part in jobs:
                if i > 0:
                    filler.add(part, 0, qkv_mm.work * 0.98)
                else:
                    filler.add(part, qkv_mm.work * (QKV_STAGES[-2] + 0.1) / qkv_mm.nq, qkv_mm.work * 0.94)
            row = lax.broadcasted_iota(I32, (KD, RB), 0)
            row8 = lax.broadcasted_iota(I32, (8, RB), 0)
            nd = D // LANE
            tiles, todo = {}, [(part, h) for part in range(3) for h in range(H)]

            def window(part, start, size, axis):
                pieces = []
                for t in range(start // LANE, (min(start + size, D) - 1) // LANE + 1):
                    a, b = max(start - t * LANE, 0), min(start + size - t * LANE, LANE)
                    pieces.append(lax.slice_in_dim(tiles[part, t], a, b, axis=axis))
                if start + size > D:
                    pieces.append(jnp.zeros_like(lax.slice_in_dim(pieces[0], 0, start + size - D, axis=axis)))
                return pieces[0] if len(pieces) == 1 else jnp.concatenate(pieces, axis=axis)

            for n, res in enumerate(qkv_mm.columns(xn.at[i % 2], xn_op.at[i % 2], wqkv, wqkv_op, filler, step, i > 0)):
                if i == 0 and n + 1 in QKV_STAGES[1:-1]:
                    qkv_stage(QKV_STAGES.index(n + 1))
                for t, val in res.items():
                    if t // nd == 0:
                        tiles[0, t % nd] = (val * QSCALE).T
                    elif t // nd == 1:
                        tiles[1, t % nd] = _pack(val)
                        if i == NB - 1:
                            tiles[3, t % nd] = val[RB - KPAD:].T
                    else:
                        tiles[2, t % nd] = val.T
                for part, h in list(todo):
                    b0 = 8 * (DH * h // 8)
                    if (part, b0 // LANE) not in tiles or (part, (min(b0 + KD, D) - 1) // LANE) not in tiles:
                        continue
                    todo.remove((part, h))
                    if part == 0:
                        lo = DH * h - b0
                        qw.at[h, i][...] = _pack(jnp.where((row >= lo) & (row < lo + DH), window(0, b0, KD, 0), 0.0))
                    elif part == 1:
                        kw[h, _half(i * RB, (i + 1) * RB), :] = window(1, b0, KD, 1)
                        if i == NB - 1:
                            kt[h] = window(3, b0, VR, 0)
                    elif h % 2 == 0:
                        vw[h, i, 0:16] = window(2, b0, 16, 0)
                        vw[h, i, 16:24] = jnp.where(row8 < 4, window(2, b0 + 16, 8, 0), 1.0)
                    else:
                        vw[h, i, 0:8] = jnp.where(row8 < 4, 1.0, window(2, b0, 8, 0))
                        vw[h, i, 8:24] = window(2, b0 + 8, 16, 0)
            assert not todo
            filler.flush()

        def first_blocks(n, carry):
            @pl.when(n == 0)
            def _():
                project(0, [norm_jobs(xv.at[1], 1, qkv_mm, xn_op, 32)], 256)

            @pl.when(n < 1)
            def _():
                for i in range(2, NB):
                    x_copy(i).wait()
                for c in other_copies:
                    c.start()

            @pl.when(n != 1)
            def _():
                for i in range(1, NB - 1):
                    project(i, [norm_jobs(xv.at[i + 1], (i + 1) % 2, qkv_mm, xn_op, 16)], 128)

            @pl.when(n + 1 == 1)
            def _():
                for c in other_copies:
                    c.wait()
            return carry

        x_copy(0).start()
        for c in qkv_copies[:2]:
            c.start()
        x_copy(0).wait()
        for c in qkv_copies[2:]:
            c.start()
        x_copy(1).start()
        for job in norm_jobs(xv.at[0], 0, qkv_mm, xn_op, 64):
            job()
        qkv_stage(0)
        lax.fori_loop(0, 2, first_blocks, 0)
        project(NB - 1, [out_mm.weight_jobs(wo, wo_op), down_mm.weight_jobs(w2, w2_op),
                         up_mm.weight_jobs(w1, w1_op)], 128)

        def attention(new, old, nxt, par, group):
            acc, pend, vacc = {}, {}, {}
            shared = old is not None

            def put(a, b, u, s):
                probs[par][_half(a, b), _lanes(u)] = _pack(jnp.exp2(s))

            def mxu_scores(c, u):
                k_ref, q_ref = new
                total = (mxu_keys + 16 * (u % 4 == 3) if shared else S) // 16
                a, b = 16 * (total * c // NT), 16 * (total * (c + 1) // NT)
                put(a, b, u, _dot(_unpack(k_ref[_half(a, b), :]), _unpack(q_ref[u // TPB, :, _lanes(u % TPB)])))

            def vpu_scores(a0, u, d):
                sums = vacc.setdefault((a0, u), [None, None])
                q = qb[par][d, :, _lanes(u)]
                for a in range(2):
                    t = kb[par][d, a0 + 8 * a:a0 + 8 * a + 8, :] * q
                    sums[a] = sums[a] + t if d else t
                if d == DH - 1:
                    put(mxu_keys + a0, mxu_keys + a0 + 16, u, jnp.concatenate(sums, axis=0))

            def fetch(c, u):
                pend[c, u] = _unpack(probs[1 - par][_half(c * LANE, (c + 1) * LANE), _lanes(u)])

            def weigh(c, u):
                v_ref, o_ref = old
                o = _dot(v_ref[c // TPB, :, _lanes(c % TPB)], pend.pop((c, u)))
                acc[u] = acc[u] + o if c else o
                if c == NT - 1:
                    o_ref[u // TPB, :, _lanes(u % TPB)] = acc[u]

            def spread_k(d):
                r = d + 4 * (1 - par)
                kb[1 - par][d] = jnp.broadcast_to(nxt[0][r:r + 1, :], (LANE, KPAD)).T[KPAD - VPU_KEYS:]

            def spread_q(u):
                q = _unpack(nxt[1][u // TPB, :, _lanes(u % TPB)]).astype(F32)
                for d in range(DH):
                    r = d + 4 * (1 - par)
                    qb[1 - par][d, :, _lanes(u)] = jnp.broadcast_to(q[r:r + 1, :], (8, LANE))

            events = []
            for j in range(NT // group):
                t0 = j * NT * group
                cells = [(t0 + c * group + w, c, j * group + w) for c in range(NT) for w in range(group)]
                pairs = [(c + k, j * group + w) for c in range(0, NT, 2) for w in range(group) for k in range(2)]
                for t, (c, u) in enumerate(pairs if old is not None else [], t0):
                    events.append((t - 4, 0, functools.partial(fetch, c, u)))
                    events.append((t, 1, functools.partial(weigh, c, u)))
                for t, c, u in cells if new is not None else []:
                    events.append((t - 3.5, 3, functools.partial(mxu_scores, c, u)))
                parts = [(a0, j * group + (w + 4) % group, d) for a0 in range(0, VPU_KEYS, 16)
                         for w in range(group) for d in range(DH) if a0 or w % 4 != 3]
                for n, part in enumerate(parts if new is not None and shared else []):
                    t = (t0 + NT * group * (n + 0.5) / len(parts)) * 98.8 / 100 + 3.5
                    events.append((t, 2, functools.partial(vpu_scores, *part)))
            if nxt is not None:
                for job, count, a, b in ((spread_k, DH, 20, 80), (spread_q, NT, 30, 80)):
                    for n in range(count):
                        events.append((NT * NT * (a + (b - a) * (n + 0.5) / count) / 100, 8, functools.partial(job, n)))
            events.sort(key=lambda e: e[:2])
            return [e[2] for e in events]

        def two_heads(j, carry):
            for par in (1, 0):
                h = 2 * j + 2 - par
                new, old, nxt = jnp.minimum(h, H - 1), h - 1, jnp.minimum(h + 1, H - 1)
                refs = (kw.at[new], qw.at[new]), (vw.at[old], oraw.at[old]), (kt.at[nxt], qw.at[nxt])

                @pl.when(h < H)
                def _():
                    for job in attention(*refs, par, NT):
                        job()
            return carry

        seen[0:2] = jnp.ones((2, 8, LANE), F32)
        seen[2] = jnp.zeros((8, LANE), F32)
        for job in attention((kw.at[0], qw.at[0]), None, (kt.at[1], qw.at[1]), 0, NT):
            job()
        lax.fori_loop(0, H // 2, two_heads, 0)

        def heads(i, u, h0, h1):
            row8 = lax.broadcasted_iota(I32, (8, LANE), 0)
            parts, sums = [], []
            for h in range(h0, h1, 2):
                e, o = oraw[h, i, :, _lanes(u)], oraw[h + 1, i, :, _lanes(u)]
                total = jnp.where(row8 < 4, o[0:8], e[16:24])
                inv = pl.reciprocal(total, approx=True)
                inv = inv * (2.0 - total * inv)
                parts += [e[0:16] * inv[4:5], jnp.where(row8 < 4, e[16:24], o[0:8]) * pltpu.roll(inv, 4, 0),
                          o[8:24] * inv[0:1]]
                sums.append(total)
            return jnp.concatenate(parts, axis=0), sums

        def gather_jobs(i, tiles):
            res, stats, n = {}, [], out_mm.rows // LANE

            def tile(u):
                h0 = tiles[0] * LANE // (2 * DH) * 2
                a, sums = heads(i, u, h0, min(H, (tiles[-1] + 1) * LANE // DH + 1))
                stats.append((functools.reduce(jnp.minimum, sums), functools.reduce(jnp.maximum, sums),
                              jnp.sum(a.reshape(-1, 8, LANE), axis=0)))
                for t in tiles:
                    res[u, t] = a[t * LANE - h0 * DH:(t + 1) * LANE - h0 * DH].T
                    att.at[i][_half(u * LANE, (u + 1) * LANE), _lanes(t)] = _pack(res[u, t])

            def operands(u, r):
                out_mm.put_input(lambda p, t: res[p * n + u, t][r:r + 32], att_op.at[i], u * LANE + r, u * LANE + r + 32)

            def record():
                lo, hi, total = zip(*stats)
                seen[0] = functools.reduce(jnp.minimum, lo, seen[0])
                seen[1] = functools.reduce(jnp.maximum, hi, seen[1])
                seen[2] = functools.reduce(jnp.add, total, seen[2])

            jobs = []
            for u in range(n):
                jobs += [functools.partial(tile, p * n + u) for p in range(out_mm.q)]
                if tiles[0] == 0:
                    jobs += [functools.partial(operands, u, r) for r in range(0, LANE, 32)]
            return jobs + [record]

        def mix(blocks, jobs, pending):
            spread = _Filler()
            spread.add(jobs, 0, out_mm.work * len(blocks) * 0.9)
            for i in blocks:
                filler = _Filler(spread)
                filler.add(gather_jobs(i, (4,)), 0, out_mm.rows * out_mm.kq * 5)
                if i == 0:
                    filler.add(pending, 0, out_mm.work * 0.85)
                if i + 1 < NB:
                    filler.add(gather_jobs(i + 1, (0, 1, 2, 3)), 0, out_mm.work * 0.95)
                for res in out_mm.columns(att.at[i], att_op.at[i], wo, wo_op, filler, 256):
                    for t, val in res.items():
                        hres[i, :, _lanes(t)] = xv[i, :, _lanes(t)].astype(F32) + val
                filler.flush()
            spread.flush()

        def project_heads(n, carry):
            @pl.when(n == 0)
            def _():
                last = attention(None, (vw.at[H - 1], oraw.at[H - 1]), None, H % 2, TPB)
                count = len(last) // NB + 8
                filler = _Filler()
                filler.add(gather_jobs(0, (0, 1, 2, 3)), 0, count)
                for job in last[:count]:
                    job()
                    filler.tick(1)
                filler.flush()
                mix(range(0, NB // 2), [], last[count:])

            @pl.when(n == 1)
            def _():
                mix(range(NB // 2, NB), norm_jobs(hres.at[0], 0, up_mm, hn_op, 16), [])
            return carry

        def feed_forward(i, carry):
            h_ref, next_ref, out_ref = hres.at[i], hres.at[jnp.minimum(i + 1, NB - 1)], xv.at[i]

            @pl.when(i != NB)
            def _():
                bias = b1[...].astype(F32).reshape(1, F)
                cols = {}
                for res in up_mm.columns(xn.at[0], hn_op.at[0], w1, w1_op, _Filler(), RB):
                    for t, val in res.items():
                        r = jnp.maximum(val + bias[:, _lanes(t)], 0.0)
                        cols[t] = r * r
                        act[:, _lanes(t)] = _pack(cols[t])
                    ready = [k for k in range(down_mm.kq) if k in cols and down_mm.kq + k in cols]
                    down_mm.put_input(lambda p, t: cols[t][p * down_mm.rows:(p + 1) * down_mm.rows],
                                      act_op.at[0], 0, down_mm.rows, ready)
                    for k in ready:
                        cols.pop(k)
                bias = b2[...].astype(F32).reshape(1, D)
                filler = _Filler()
                filler.add(norm_jobs(next_ref, 0, up_mm, hn_op, 16), 0, down_mm.work * 0.9)
                for res in down_mm.columns(act, act_op.at[0], w2, w2_op, filler, RB // 2):
                    for t, val in res.items():
                        out_ref[:, _lanes(t)] = (h_ref[:, _lanes(t)] + (val + bias[:, _lanes(t)])).astype(BF16)
                        o_copy(i, t).start()
                filler.flush()
            return carry

        lax.fori_loop(0, 2, project_heads, 0)
        lax.fori_loop(0, NB, feed_forward, 0)
        safe = (seen[0] >= SUM_MIN) & (seen[1] <= SUM_MAX) & (jnp.abs(seen[2]) <= 3e38)
        unsafe = jnp.max(jnp.where(safe, 0, 1)) > 0
        for i in range(NB):
            for t in range(D // LANE):
                o_copy(i, t).wait()

        @pl.when(unsafe)
        def _():
            def head(n, carry):
                h, i = n // NB, n % NB
                q = _unpack(qw[h, i])

                def scores(c):
                    rows = pl.ds(pl.multiple_of(c * (LANE // 2), LANE // 2), LANE // 2)
                    return _dot(_unpack(kw[h, rows, :]), q)

                m = lax.fori_loop(0, NT, lambda c, m: jnp.maximum(m, jnp.max(scores(c), axis=0, keepdims=True)),
                                  jnp.full((1, RB), -jnp.inf, F32))

                def weigh(b, o):
                    for c in range(TPB):
                        o = o + _dot(vw[h, b, :, _lanes(c)], jnp.exp2(scores(b * TPB + c) - m))
                    return o
                oraw[h, i] = lax.fori_loop(0, NB, weigh, jnp.zeros((VR, RB), F32))
                return carry
            lax.fori_loop(0, H * NB, head, 0)

            def block(i, carry):
                x_copy(i).start()
                x_copy(i).wait()
                for u in range(TPB):
                    att.at[0][_half(u * LANE, (u + 1) * LANE), :] = _pack(heads(i, u, 0, H)[0].T)

                def rows(r, carry):
                    at = pl.ds(pl.multiple_of(r * 32, 32), 32)
                    a = _unpack(att[0, pl.ds(pl.multiple_of(r * 16, 16), 16), :])
                    hh = xv[i, at, :].astype(F32) + _dot(a, wo[...])
                    g = jnp.maximum(_dot(_ln(hh).astype(BF16), w1[...]) + b1[...].astype(F32).reshape(1, F), 0.0)
                    out = hh + (_dot((g * g).astype(BF16), w2[...]) + b2[...].astype(F32).reshape(1, D))
                    xv[i, at, :] = out.astype(BF16)
                    return carry
                lax.fori_loop(0, RB // 32, rows, 0)
                done = pltpu.make_async_copy(xv.at[i], o_hbm.at[pl.ds(i * RB, RB)], sem_x.at[i])
                done.start()
                done.wait()
                return carry
            lax.fori_loop(0, NB, block, 0)

    scratch = [
        pltpu.VMEM((NB, RB, D), BF16),
        pltpu.VMEM((D, 3 * D), BF16), pltpu.VMEM((D, D), BF16), pltpu.VMEM((D, F), BF16), pltpu.VMEM((F, D), BF16),
        qkv_mm.weight_scratch(), out_mm.weight_scratch(), up_mm.weight_scratch(), down_mm.weight_scratch(),
        pltpu.VMEM((2, RB // 2, D), I32), qkv_mm.input_scratch(2), up_mm.input_scratch(1),
        pltpu.VMEM((NB, RB // 2, D), I32), out_mm.input_scratch(NB),
        pltpu.VMEM((RB // 2, F), I32), down_mm.input_scratch(1),
        pltpu.VMEM((NB, RB, D), F32),
        pltpu.VMEM((H, S // 2, KD), I32), pltpu.VMEM((H, VR, KPAD), F32),
        pltpu.VMEM((H, NB, KD // 2, RB), I32),
        pltpu.VMEM((H, NB, VR, RB), F32), pltpu.VMEM((H, NB, VR, RB), F32),
        pltpu.VMEM((4, 8, LANE), F32),
        pltpu.VMEM((S // 2, S), I32), pltpu.VMEM((S // 2, S), I32),
        pltpu.VMEM((DH, VPU_KEYS, LANE), F32), pltpu.VMEM((DH, VPU_KEYS, LANE), F32),
        pltpu.VMEM((DH, 8, S), F32), pltpu.VMEM((DH, 8, S), F32),
        pltpu.VMEM((F,), BF16), pltpu.VMEM((D,), BF16),
        pltpu.SemaphoreType.DMA((NB,)), pltpu.SemaphoreType.DMA((2 * len(QKV_STAGES) + 3,)), pltpu.SemaphoreType.DMA((NB * D // LANE,)),
    ]
    out = pl.pallas_call(
        kernel,
        out_shape=jax.ShapeDtypeStruct((S, D), BF16),
        in_specs=[pl.BlockSpec(memory_space=pl.ANY)] * 7,
        out_specs=pl.BlockSpec(memory_space=pl.ANY),
        scratch_shapes=scratch,
        compiler_params=pltpu.CompilerParams(
            vmem_limit_bytes=120 * 2**20, flags={"XLA_TPU_EVENLY_DISTRIBUTE_CRITICAL_NODES": True}),
    )(A_x.reshape(S, D), A_wqkv, A_wo, B_w1, B_b1, B_w2, B_b2)
    return out.reshape(1, S, D)
```
